```python
import jax
import jax.numpy as jnp

def _softmax(x, axis=-1):
    return jax.nn.softmax(x, axis=axis)

def _gelu(x):
    return jax.nn.gelu(x, approximate=True)

def _silu(x):
    return jax.nn.silu(x)

def _sigmoid(x):
    return jax.nn.sigmoid(x)

def _layernorm(x, axis=-1, eps=1e-05):
    m = jnp.mean(x, axis=axis, keepdims=True)
    v = jnp.var(x, axis=axis, keepdims=True)
    return (x - m) / jnp.sqrt(v + eps)

def _scatter_add(tgt, idx, src, axis=0):
    return tgt.at[idx].add(src)

def _segment_sum(src, seg, n):
    return jax.ops.segment_sum(src, seg, n)

class _Rng:

    def __init__(self, key):
        self._k = key

    def _next(self):
        self._k, sub = jax.random.split(self._k)
        return sub

    def normal(self, shape):
        return jax.random.normal(self._next(), shape, dtype=jnp.bfloat16)

    def randint(self, lo, hi, shape):
        return jax.random.randint(self._next(), shape, lo, hi, dtype=jnp.int32)

    def uniform(self, shape, lo=0.0, hi=1.0):
        return jax.random.uniform(self._next(), shape, jnp.bfloat16, lo, hi)

    def permutation(self, n):
        return jax.random.permutation(self._next(), n)
kernel_name = 'adaLN_cond__grouped_kv_mqa__dense_activation_silu__prompt'

def _fwd_setup_inputs():
    _rng = _Rng(jax.random.key(int.from_bytes(__import__("os").urandom(4), "little")))
    _w = lambda a: (lambda t: t.astype(jnp.bfloat16) if jnp.issubdtype(t.dtype, jnp.floating) else t)(jnp.asarray(a))

    def _A_setup():
        B, S, D, H = (1, 2048, 640, 32)
        Dh = D // H
        return {'x': _w((lambda *s: _rng.normal(s) * 0.05)(B, S, D)), 'wq': _w((lambda *s: _rng.normal(s) * 0.05)(D, H * Dh)), 'wk': _w((lambda *s: _rng.normal(s) * 0.05)(D, Dh)), 'wv': _w((lambda *s: _rng.normal(s) * 0.05)(D, Dh)), 'wo': _w((lambda *s: _rng.normal(s) * 0.05)(H * Dh, D))}
    _A_in = _A_setup()

    def _B_setup():
        B, S, D, F = (1, 2048, 640, 1728)
        return {'x': _w((lambda *s: _rng.normal(s) * 0.05)(B, S, D)), 'w1': _w((lambda *s: _rng.normal(s) * 0.05)(D, F) * D ** (-0.5)), 'w2': _w((lambda *s: _rng.normal(s) * 0.05)(F, D) * F ** (-0.5))}
    _B_in = _B_setup()
    return {'A_x': _A_in['x'], 'A_wq': _A_in['wq'], 'A_wk': _A_in['wk'], 'A_wv': _A_in['wv'], 'A_wo': _A_in['wo'], 'B_x': _B_in['x'], 'B_w1': _B_in['w1'], 'B_w2': _B_in['w2'], 'c': _w((lambda *s: _rng.normal(s) * 0.05)(1, 640)), 'w_mod': _w((lambda *s: _rng.normal(s) * 0.05)(640, 6 * 640) * 640 ** (-0.5))}

def _fwd_reference(A_x, A_wq, A_wk, A_wv, A_wo, B_x, B_w1, B_w2, c, w_mod):

    def _A_ref(x, wq, wk, wv, wo):
        B, S, D = x.shape
        H = 32
        Dh = D // H
        q = (lambda x, *d: x.transpose(*d))((x @ wq).reshape(B, S, H, Dh), 0, 2, 1, 3)
        k = x @ wk
        v = x @ wv
        scores = jnp.einsum('bhqd,bkd->bhqk', q, k) * Dh ** (-0.5)
        p = _softmax(scores, axis=-1)
        o = jnp.einsum('bhqk,bkd->bhqd', p, v)
        return (lambda x, *d: x.transpose(*d))(o, 0, 2, 1, 3).reshape(B, S, H * Dh) @ wo

    def _B_ref(x, w1, w2):
        h = jnp.einsum('bsd,df->bsf', x, w1)
        h = _silu(h)
        out = jnp.einsum('bsf,fd->bsd', h, w2)
        return out
    x = A_x
    mod = (_silu(c) @ w_mod).reshape(c.shape[0], 6, 1, -1)
    sa, ca, ga, sb, cb, gb = (mod[:, 0].copy(), mod[:, 1].copy(), mod[:, 2].copy(), mod[:, 3].copy(), mod[:, 4].copy(), mod[:, 5].copy())
    h = _layernorm(x, axis=-1) * (1 + ca) + sa
    x = x + ga * _A_ref(h, A_wq, A_wk, A_wv, A_wo)
    h = _layernorm(x, axis=-1) * (1 + cb) + sb
    x = x + gb * _B_ref(h, B_w1, B_w2)
    return x

def setup_inputs():
    _inp = _fwd_setup_inputs()
    _gk = jax.random.fold_in(jax.random.key(int.from_bytes(__import__("os").urandom(4), "little")), 2 ** 31 - 1)
    _shapes = [[1, 2048, 640]]
    _dtypes = ['bfloat16']
    _gks = jax.random.split(_gk, len(_shapes))
    _gs = [jax.random.normal(k, s, dtype=jnp.dtype(d)) * 0.05 for k, s, d in zip(_gks, _shapes, _dtypes)]
    _inp['grad_out'] = _gs[0]
    return _inp

def reference(A_x, A_wq, A_wk, A_wv, A_wo, B_w1, B_w2, c, w_mod, B_x, grad_out):
    _const = dict(B_x=B_x)

    def _f(*_d):
        return _fwd_reference(**{'A_x': _d[0], 'A_wq': _d[1], 'A_wk': _d[2], 'A_wv': _d[3], 'A_wo': _d[4], 'B_w1': _d[5], 'B_w2': _d[6], 'c': _d[7], 'w_mod': _d[8], **_const})
    _out, _vjp = jax.vjp(_f, A_x, A_wq, A_wk, A_wv, A_wo, B_w1, B_w2, c, w_mod)
    _grads = _vjp(grad_out)
    _out0 = jnp.asarray(_out)
    return (_out0, *[jnp.asarray(_g) for _g in _grads])
```

```python
import functools
import math

import jax
import jax.numpy as jnp
import jax.experimental.pallas as pl
import jax.experimental.pallas.tpu as pltpu

F32 = jnp.float32
BF16 = jnp.bfloat16
U32 = jnp.uint32

S = 2048
D = 640
H = 32
DH = 20
FF = 1728
FP = 1792
FC = 256
EPS = 1e-5

TQ = 256
NB = S // TQ
HP = 2
NG = H // HP
GR = HP * DH
VQ = HP * TQ
CKF = 128
CKB = 256
HD = 32

LOG2E = 1.4426950408889634
SCALE = DH ** (-0.5)

_NT = (((1,), (1,)), ((), ()))


def _dot(a, b):
    return jnp.dot(a, b, preferred_element_type=F32)


def _dot_nt(a, b):
    return jax.lax.dot_general(a, b, _NT, preferred_element_type=F32)


def _ld(v):
    return pltpu.bitcast(v, BF16)


def _pk(v):
    return pltpu.bitcast(v, U32)


def _eye(n, dtype=BF16):
    r = jax.lax.broadcasted_iota(jnp.int32, (n, n), 0)
    c = jax.lax.broadcasted_iota(jnp.int32, (n, n), 1)
    return jnp.where(r == c, 1.0, 0.0).astype(dtype)


def _sigmoid(x):
    return 0.5 * jnp.tanh(0.5 * x) + 0.5


def _wide(col, n):
    reps = n // 128
    if reps == 1:
        return col
    return jnp.concatenate([col] * reps, axis=1)


def _fold(a):
    n = a.shape[1] // 128
    acc = a[:, 0:128]
    for t in range(1, n):
        acc = acc + a[:, t * 128:(t + 1) * 128]
    return acc


def _kernel(x_hbm, wq_hbm, wkT_ref, wvT_ref, wo_hbm, w1T_hbm, w2_hbm, c_ref, wmod_hbm, g_ref,
            out_ref, dx_hbm, dwq_hbm, dwkT_ref, dwvT_ref, dwo_hbm, dw1T_hbm, dw2_hbm, dc_ref, dwmod_hbm,
            sx, swq, swo, sw1, sw2, swm, sems,
            xT, st1, h1T, modc, wqT, wqN, woT, woN, w1T, w1N, w2T, w2N, wkv,
            Kaug, Vaug, KT, VT, Qs, QB, dOs, OT, dQT, SA, SB, mA, mB, P, linv_s, dKT, dVT,
            aW1, aW2, aWq, aWo, macc, dx2T, dh1T, h2s, dfs, facc, hacc, zs):
    i = pl.program_id(0)

    in_pairs = [(wmod_hbm, swm), (x_hbm, sx), (wq_hbm, swq), (wo_hbm, swo), (w1T_hbm, sw1), (w2_hbm, sw2)]

    def in_copy(k):
        return pltpu.make_async_copy(in_pairs[k][0], in_pairs[k][1], sems.at[k])

    out_pairs = [(swm, dwmod_hbm), (sx, dx_hbm), (swq, dwq_hbm), (swo, dwo_hbm), (sw1, dw1T_hbm), (sw2, dw2_hbm)]

    def out_copy(k):
        return pltpu.make_async_copy(out_pairs[k][0], out_pairs[k][1], sems.at[6 + k])

    def transpose_into(dst, src_ref, ncols):
        eye = _eye(128)
        for c0 in range(0, ncols, 128):
            w = min(128, ncols - c0)
            e = eye if w == 128 else _eye(w)
            src = src_ref[:, c0:c0 + w]
            dst[c0 // 2:(c0 + w) // 2, 0:src.shape[0]] = _pk(_dot_nt(e, src).astype(BF16))

    def repack_into(dst, src_ref, nrows):
        for r0 in range(0, nrows, 64):
            dst[r0 // 2:(r0 + 64) // 2, :] = _pk(src_ref[r0:r0 + 64, :])

    def score_pass(n, Snext, mnext, c, m8):
        c0 = c * CKF
        z = pl.multiple_of(zs[0], 8)
        qT = _ld(QB[n])
        s = _dot(_ld(Kaug[c0 // 2:(c0 + CKF) // 2, :]), qT)
        Snext[pl.ds(z + c0, CKF), :] = s
        mc = jnp.max(s.reshape(CKF // 8, 8, VQ), axis=0)
        return mc if m8 is None else jnp.maximum(m8, mc)

    @pl.when(i == 0)
    @jax.named_scope('prologue')
    def _prologue():
        for k in range(6):
            in_copy(k).start()
        zs[0] = 0

        macc[...] = jnp.zeros_like(macc)
        dKT[...] = jnp.zeros_like(dKT)
        dVT[...] = jnp.zeros_like(dVT)
        aW1[...] = jnp.zeros_like(aW1)
        aW2[...] = jnp.zeros_like(aW2)
        aWq[...] = jnp.zeros_like(aWq)
        aWo[...] = jnp.zeros_like(aWo)
        Qs[D:D + 16, :] = jnp.zeros((16, TQ), F32)
        w1T[FF // 2:FP // 2, :] = jnp.zeros(((FP - FF) // 2, D), U32)
        w2N[FF // 2:FP // 2, :] = jnp.zeros(((FP - FF) // 2, D), U32)
        w1N[:, FP - 128:FP] = jnp.zeros((D // 2, 128), U32)
        w2T[:, FP - 128:FP] = jnp.zeros((D // 2, 128), U32)

        z12 = jnp.zeros((HD - DH, D), F32)
        wkvT = jnp.concatenate([wkT_ref[...].astype(F32), z12, wvT_ref[...].astype(F32), z12],
                               axis=0).astype(BF16)
        eye128 = _eye(128)
        for c0 in range(0, D, 128):
            wkv[c0 // 2:(c0 + 128) // 2, :] = _pk(_dot_nt(eye128, wkvT[:, c0:c0 + 128]).astype(BF16))

        cf = c_ref[...].astype(F32)
        sc = cf * _sigmoid(cf)
        scb = jnp.broadcast_to(sc, (16, D)).astype(BF16)
        in_copy(0).wait()
        mod = _dot(scb, swm[...])
        for k in range(6):
            row = mod[0:1, k * D:(k + 1) * D]
            if k in (1, 4):
                row = row + 1.0
            modc[k] = jnp.transpose(jnp.broadcast_to(row, (128, D)))

        in_copy(1).wait()
        transpose_into(xT, sx, D)

        sa = modc[0]
        ca1 = modc[1]
        rowid = jax.lax.broadcasted_iota(jnp.int32, (HD, 128), 0)
        ones_rows = jnp.logical_and(rowid >= DH, rowid < DH + 2)

        def ln1_body(t, carry):
            t0 = pl.multiple_of(t * 128, 128)
            xt = _ld(xT[:, pl.ds(t0, 128)]).astype(F32)
            mu = jnp.mean(xt, axis=0, keepdims=True)
            xc = xt - mu
            var = jnp.mean(xc * xc, axis=0, keepdims=True)
            rstd = jax.lax.rsqrt(var + EPS)
            st1[0:1, pl.ds(t0, 128)] = mu
            st1[1:2, pl.ds(t0, 128)] = rstd
            h1 = (xc * rstd * ca1 + sa).astype(BF16)
            h1T[:, pl.ds(t0, 128)] = _pk(h1)
            kv = _dot(wkvT, h1)
            kt = kv[0:HD].astype(BF16)
            vt = jnp.where(ones_rows, 1.0, kv[HD:2 * HD]).astype(BF16)
            KT[:, pl.ds(t0, 128)] = _pk(kt)
            VT[:, pl.ds(t0, 128)] = _pk(vt)
            r0 = pl.multiple_of(t * 64, 64)
            Kaug[pl.ds(r0, 64), :] = _pk(_dot_nt(eye128, kt).astype(BF16))
            Vaug[pl.ds(r0, 64), :] = _pk(_dot_nt(eye128, vt).astype(BF16))
            return carry

        jax.lax.fori_loop(0, S // 128, ln1_body, 0)

        in_copy(2).wait()
        transpose_into(wqT, swq, D)
        repack_into(wqN, swq, D)

        def q_body(b, carry):
            t0 = pl.multiple_of(b * TQ, TQ)
            Qs[0:D, :] = _dot(_ld(wqT[...]), _ld(h1T[:, pl.ds(t0, TQ)])) * (SCALE * LOG2E)
            for g in range(NG):
                qblk = Qs[g * GR:g * GR + GR + 16, :]
                qT = jnp.concatenate([qblk[0:HD], qblk[DH:DH + HD]], axis=1).astype(BF16)
                QB[b * NG + g] = _pk(qT)
            return carry

        jax.lax.fori_loop(0, NB, q_body, 0)

        m8 = None
        for c in range(S // CKF):
            m8 = score_pass(0, SA, mA, c, m8)
        mA[...] = jnp.broadcast_to(jnp.max(m8, axis=0, keepdims=True), (8, VQ))

        in_copy(3).wait()
        transpose_into(woT, swo, D)
        repack_into(woN, swo, D)
        in_copy(4).wait()
        repack_into(w1T, sw1, FF)
        transpose_into(w1N, sw1, D)
        in_copy(5).wait()
        repack_into(w2N, sw2, FF)
        transpose_into(w2T, sw2, D)

    t0 = pl.multiple_of(i * TQ, TQ)

    def fwd_step(g, n, Scur, mcur, Snext, mnext):
        m = mcur[0:1, :]
        z = pl.multiple_of(zs[0], 8)
        m8 = None
        acc = None
        for c in range(S // CKF):
            c0 = c * CKF
            m8 = score_pass(n, Snext, mnext, c, m8)
            p = jnp.exp2(Scur[pl.ds(z + c0, CKF), :] - m).astype(BF16)
            P[g, c0 // 2:(c0 + CKF) // 2, :] = _pk(p)
            r = _dot(_ld(VT[:, c0:c0 + CKF]), p)
            acc = r if acc is None else acc + r
        mnext[...] = jnp.broadcast_to(jnp.max(m8, axis=0, keepdims=True), (8, VQ))
        linv = 1.0 / acc[DH:DH + 1, :]
        linv_s[g] = jnp.broadcast_to(linv, (8, VQ))
        o = acc[0:DH, :] * linv
        r0 = pl.multiple_of(g * GR, 8)
        OT[pl.ds(r0, GR), :] = jnp.concatenate([o[:, 0:TQ], o[:, TQ:VQ]], axis=0)

    def fwd_body(gg, carry):
        g = 2 * gg
        n = i * NG + g
        fwd_step(g, n + 1, SA, mA, SB, mB)
        fwd_step(g + 1, jnp.minimum(n + 2, NB * NG - 1), SB, mB, SA, mA)
        return carry

    with jax.named_scope('fwdloop'):
        jax.lax.fori_loop(0, NG // 2, fwd_body, 0)

    with jax.named_scope('mid1'):
        ga = _wide(modc[2], TQ)
        sb = _wide(modc[3], TQ)
        cb1 = _wide(modc[4], TQ)
        gb = _wide(modc[5], TQ)
        eye128 = _eye(128)

        gT = jnp.concatenate(
            [_dot_nt(eye128, g_ref[:, c0:c0 + 128]) for c0 in range(0, D, 128)], axis=0)
        dfs[...] = _pk((gT * gb).astype(BF16))

        OTb = OT[...].astype(BF16)
        attn = _dot(_ld(woT[...]), OTb)
        x2 = _ld(xT[:, pl.ds(t0, TQ)]).astype(F32) + ga * attn
        mu2 = jnp.mean(x2, axis=0, keepdims=True)
        xc2 = x2 - mu2
        var2 = jnp.mean(xc2 * xc2, axis=0, keepdims=True)
        rstd2 = jax.lax.rsqrt(var2 + EPS)
        xh2 = xc2 * rstd2
        h2s[...] = _pk((xh2 * cb1 + sb).astype(BF16))
        facc[...] = jnp.zeros_like(facc)
        hacc[...] = jnp.zeros_like(hacc)

    def ffn_body(j, carry):
        f0 = pl.multiple_of(j * FC, FC)
        r0 = pl.multiple_of(j * (FC // 2), FC // 2)
        h2 = _ld(h2s[...])
        df = _ld(dfs[...])
        u = _dot(_ld(w1T[pl.ds(r0, FC // 2), :]), h2)
        da = _dot(_ld(w2N[pl.ds(r0, FC // 2), :]), df)
        sg = _sigmoid(u)
        a = (u * sg).astype(BF16)
        du = (da * (sg * (1.0 + u * (1.0 - sg)))).astype(BF16)
        facc[...] += _dot(_ld(w2T[:, pl.ds(f0, FC)]), a)
        aW2[pl.ds(f0, FC), :] += _dot_nt(a, df)
        hacc[...] += _dot(_ld(w1N[:, pl.ds(f0, FC)]), du)
        aW1[pl.ds(f0, FC), :] += _dot_nt(du, h2)
        return carry

    with jax.named_scope('ffnloop'):
        jax.lax.fori_loop(0, FP // FC, ffn_body, 0)

    with jax.named_scope('mid2'):
        f = facc[...]
        outT = (x2 + gb * f).astype(BF16)
        for c0 in range(0, TQ, 128):
            out_ref[c0:c0 + 128, :] = _dot_nt(eye128, outT[:, c0:c0 + 128]).astype(BF16)
        macc[5] += _fold(gT * f)
        dh2 = hacc[...]
        macc[4] += _fold(dh2 * xh2)
        macc[3] += _fold(dh2)
        dxh = dh2 * cb1
        m1 = jnp.mean(dxh, axis=0, keepdims=True)
        m2 = jnp.mean(dxh * xh2, axis=0, keepdims=True)
        dx2 = gT + rstd2 * (dxh - m1 - xh2 * m2)
        dx2T[:, pl.ds(t0, TQ)] = dx2
        macc[2] += _fold(dx2 * attn)
        dattn = (dx2 * ga).astype(BF16)
        dOs[...] = _dot(_ld(woN[...]), dattn)
        aWo[...] += _dot_nt(OTb, dattn)

    @pl.when(i == NB - 1)
    @jax.named_scope('earlyout')
    def _early_out():
        swo[...] = aWo[...].astype(BF16)
        sw1[...] = aW1[0:FF, :].astype(BF16)
        sw2[...] = aW2[0:FF, :].astype(BF16)
        out_copy(3).start()
        out_copy(4).start()
        out_copy(5).start()

    def bwd_group(g, carry):
        r0 = pl.multiple_of(g * GR, 8)
        dob = dOs[pl.ds(r0, GR), :]
        ob = OT[pl.ds(r0, GR), :]
        do = jnp.concatenate([dob[0:DH], dob[DH:GR]], axis=1)
        o = jnp.concatenate([ob[0:DH], ob[DH:GR]], axis=1)
        linv = linv_s[g][0:1, :]
        nd = -jnp.sum(do * o, axis=0, keepdims=True) * linv
        nd_hi = nd.astype(BF16).astype(F32)
        nd_lo = nd - nd_hi
        W = jnp.concatenate([do * linv, nd_hi, nd_lo, jnp.zeros((HD - DH - 2, VQ), F32)],
                            axis=0).astype(BF16)
        qT = _ld(QB[i * NG + g])
        dq = None
        prev = None
        nch = S // CKB
        H2 = CKB // 2
        for c in range(nch + 1):
            c0 = c * CKB
            if c < nch:
                dpa = _dot(_ld(Vaug[c0 // 2:(c0 + H2) // 2, :]), W)
            if prev is not None:
                pc0, pds, pp = prev
                dKT[:, pc0:pc0 + CKB] += _dot_nt(qT, pds)
            if c < nch:
                dpb = _dot(_ld(Vaug[(c0 + H2) // 2:(c0 + CKB) // 2, :]), W)
            if prev is not None:
                dVT[:, pc0:pc0 + CKB] += _dot_nt(W, pp)
                r = _dot(_ld(KT[:, pc0:pc0 + CKB]), pds)
                dq = r if dq is None else dq + r
            if c < nch:
                p = _ld(P[g, c0 // 2:(c0 + CKB) // 2, :])
                pf = p.astype(F32)
                ds = jnp.concatenate([(pf[:H2] * dpa).astype(BF16), (pf[H2:] * dpb).astype(BF16)], axis=0)
                prev = (c0, ds, p)
        dq = dq[0:DH, :] * SCALE
        dQT[pl.ds(r0, GR), :] = jnp.concatenate([dq[:, 0:TQ], dq[:, TQ:VQ]], axis=0)
        return carry

    with jax.named_scope('bwdloop'):
        jax.lax.fori_loop(0, NG, bwd_group, 0)

    with jax.named_scope('post'):
        dQb = dQT[...].astype(BF16)
        dh1T[:, pl.ds(t0, TQ)] = _dot(_ld(wqN[...]), dQb)
        aWq[...] += _dot_nt(_ld(h1T[:, pl.ds(t0, TQ)]), dQb)

    @pl.when(i == NB - 1)
    @jax.named_scope('epilogue')
    def _epilogue():
        swq[...] = aWq[...].astype(BF16)
        out_copy(2).start()
        dkv = jnp.concatenate([dKT[...] * (1.0 / LOG2E), dVT[...]], axis=0).astype(BF16)
        dwkvT = _dot_nt(dkv, _ld(h1T[...]))
        dwkT_ref[...] = dwkvT[0:DH].astype(BF16)
        dwvT_ref[...] = dwkvT[HD:HD + DH].astype(BF16)
        KT[...] = _pk(dkv[0:HD])
        VT[...] = _pk(dkv[HD:2 * HD])
        ca1 = modc[1]
        eye = _eye(128)

        def ln1b_body(t, carry):
            c0 = pl.multiple_of(t * 128, 128)
            dkvc = jnp.concatenate([_ld(KT[:, pl.ds(c0, 128)]), _ld(VT[:, pl.ds(c0, 128)])], axis=0)
            dh1 = dh1T[:, pl.ds(c0, 128)] + _dot(_ld(wkv[...]), dkvc)
            mu = st1[0:1, pl.ds(c0, 128)]
            rstd = st1[1:2, pl.ds(c0, 128)]
            xh = (_ld(xT[:, pl.ds(c0, 128)]).astype(F32) - mu) * rstd
            macc[1] += dh1 * xh
            macc[0] += dh1
            dxh1 = dh1 * ca1
            n1 = jnp.mean(dxh1, axis=0, keepdims=True)
            n2 = jnp.mean(dxh1 * xh, axis=0, keepdims=True)
            dxt = (dx2T[:, pl.ds(c0, 128)] + rstd * (dxh1 - n1 - xh * n2)).astype(BF16)
            sx[pl.ds(c0, 128), :] = _dot_nt(eye, dxt).astype(BF16)
            return carry

        jax.lax.fori_loop(0, S // 128, ln1b_body, 0)
        out_copy(1).start()

        cf = c_ref[...].astype(F32)
        sgc = _sigmoid(cf)
        sc = cf * sgc
        scc = jnp.transpose(jnp.broadcast_to(sc, (128, D)))
        rows = [jnp.sum(jnp.transpose(macc[k]), axis=0, keepdims=True) for k in range(6)]
        dmod = jnp.concatenate(rows, axis=1)
        hi = dmod.astype(BF16).astype(F32)
        lo = dmod - hi
        rid = jax.lax.broadcasted_iota(jnp.int32, (16, 6 * D), 0)
        lhs = jnp.where(rid == 0, hi, jnp.where(rid == 1, lo, 0.0)).astype(BF16)
        dsc2 = _dot_nt(lhs, swm[...])
        dsc = dsc2[0:1] + dsc2[1:2]
        dc_ref[...] = (dsc * (sgc * (1.0 + cf * (1.0 - sgc)))).astype(BF16)
        for k in range(6):
            swm[:, k * D:(k + 1) * D] = (_wide(scc, D) * rows[k]).astype(BF16)
        out_copy(0).start()
        for k in range(6):
            out_copy(k).wait()


@jax.jit
def pallas_adaLN_cond__grouped_kv_mqa__dense_activation_silu__prompt_kernel(
    A_x: jax.Array,
    A_wq: jax.Array,
    A_wk: jax.Array,
    A_wv: jax.Array,
    A_wo: jax.Array,
    B_x: jax.Array,
    B_w1: jax.Array,
    B_w2: jax.Array,
    c: jax.Array,
    w_mod: jax.Array,
    grad_out: jax.Array,
):
    x = A_x.reshape(S, D)
    g = grad_out.reshape(S, D)

    def full(shape):
        return pl.BlockSpec(shape, lambda i: (0,) * len(shape))

    hbm = pl.BlockSpec(memory_space=pl.ANY)

    in_specs = [
        hbm, hbm, full((DH, D)), full((DH, D)), hbm,
        hbm, hbm, full((1, D)), hbm,
        pl.BlockSpec((TQ, D), lambda i: (i, 0)),
    ]
    out_specs = [
        pl.BlockSpec((TQ, D), lambda i: (i, 0)),
        hbm, hbm, full((DH, D)), full((DH, D)), hbm,
        hbm, hbm, full((1, D)), hbm,
    ]
    out_shape = [
        jax.ShapeDtypeStruct((S, D), BF16), jax.ShapeDtypeStruct((S, D), BF16),
        jax.ShapeDtypeStruct((D, D), BF16), jax.ShapeDtypeStruct((DH, D), BF16),
        jax.ShapeDtypeStruct((DH, D), BF16), jax.ShapeDtypeStruct((D, D), BF16),
        jax.ShapeDtypeStruct((FF, D), BF16), jax.ShapeDtypeStruct((FF, D), BF16),
        jax.ShapeDtypeStruct((1, D), BF16), jax.ShapeDtypeStruct((D, 6 * D), BF16),
    ]
    scratch = [
        pltpu.VMEM((S, D), BF16),
        pltpu.VMEM((D, D), BF16),
        pltpu.VMEM((D, D), BF16),
        pltpu.VMEM((FF, D), BF16),
        pltpu.VMEM((FF, D), BF16),
        pltpu.VMEM((D, 6 * D), BF16),
        pltpu.SemaphoreType.DMA((12,)),
        pltpu.VMEM((D // 2, S), U32),
        pltpu.VMEM((8, S), F32),
        pltpu.VMEM((D // 2, S), U32),
        pltpu.VMEM((6, D, 128), F32),
        pltpu.VMEM((D // 2, D), U32),
        pltpu.VMEM((D // 2, D), U32),
        pltpu.VMEM((D // 2, D), U32),
        pltpu.VMEM((D // 2, D), U32),
        pltpu.VMEM((FP // 2, D), U32),
        pltpu.VMEM((D // 2, FP), U32),
        pltpu.VMEM((D // 2, FP), U32),
        pltpu.VMEM((FP // 2, D), U32),
        pltpu.VMEM((D // 2, 2 * HD), U32),
        pltpu.VMEM((S // 2, HD), U32),
        pltpu.VMEM((S // 2, HD), U32),
        pltpu.VMEM((HD // 2, S), U32),
        pltpu.VMEM((HD // 2, S), U32),
        pltpu.VMEM((D + 16, TQ), F32),
        pltpu.VMEM((NB * NG, HD // 2, VQ), U32),
        pltpu.VMEM((D, TQ), F32),
        pltpu.VMEM((D, TQ), F32),
        pltpu.VMEM((D, TQ), F32),
        pltpu.VMEM((S, VQ), F32),
        pltpu.VMEM((S, VQ), F32),
        pltpu.VMEM((8, VQ), F32),
        pltpu.VMEM((8, VQ), F32),
        pltpu.VMEM((NG, S // 2, VQ), U32),
        pltpu.VMEM((NG, 8, VQ), F32),
        pltpu.VMEM((HD, S), F32),
        pltpu.VMEM((HD, S), F32),
        pltpu.VMEM((FP, D), F32),
        pltpu.VMEM((FP, D), F32),
        pltpu.VMEM((D, D), F32),
        pltpu.VMEM((D, D), F32),
        pltpu.VMEM((6, D, 128), F32),
        pltpu.VMEM((D, S), F32),
        pltpu.VMEM((D, S), F32),
        pltpu.VMEM((D // 2, TQ), U32),
        pltpu.VMEM((D // 2, TQ), U32),
        pltpu.VMEM((D, TQ), F32),
        pltpu.VMEM((D, TQ), F32),
        pltpu.SMEM((1,), jnp.int32),
    ]
    outs = pl.pallas_call(
        _kernel,
        grid=(NB,),
        in_specs=in_specs,
        out_specs=out_specs,
        out_shape=out_shape,
        scratch_shapes=scratch,
        compiler_params=pltpu.CompilerParams(
            dimension_semantics=("arbitrary",),
            vmem_limit_bytes=126 * 1024 * 1024,
        ),
    )(x, A_wq, A_wk.T, A_wv.T, A_wo, B_w1.T, B_w2, c, w_mod, g)
    out, dx, dwq, dwkT, dwvT, dwo, dw1T, dw2, dc, dwmod = outs
    return (out.reshape(1, S, D), dx.reshape(1, S, D), dwq, dwkT.T, dwvT.T, dwo, dw1T.T, dw2, dc, dwmod)
```

```python
import functools
import math

import jax
import jax.numpy as jnp
import jax.experimental.pallas as pl
import jax.experimental.pallas.tpu as pltpu

F32 = jnp.float32
BF16 = jnp.bfloat16
U32 = jnp.uint32

S = 2048
D = 640
H = 32
DH = 20
FF = 1728
FC = 864
NFC = FF // FC
FCP = 896
FS = 288
EPS = 1e-5

TQ = 256
NB = S // TQ
HP = 2
NG = H // HP
GR = HP * DH
VQ = HP * TQ
CKF = 128
CKB = 256
HD = 32
UF = 2
UB = 4
SKEW = 1
LW = 512

LOG2E = 1.4426950408889634
SCALE = DH ** (-0.5)

_NT = (((1,), (1,)), ((), ()))


def _dot(a, b):
    return jnp.dot(a, b, preferred_element_type=F32)


def _dot_nt(a, b):
    return jax.lax.dot_general(a, b, _NT, preferred_element_type=F32)


def _ld(v):
    return pltpu.bitcast(v, BF16)


def _pk(v):
    return pltpu.bitcast(v, U32)


def _eye(n, dtype=BF16):
    r = jax.lax.broadcasted_iota(jnp.int32, (n, n), 0)
    c = jax.lax.broadcasted_iota(jnp.int32, (n, n), 1)
    return jnp.where(r == c, 1.0, 0.0).astype(dtype)


def _sigmoid(x):
    return 0.5 * jnp.tanh(0.5 * x) + 0.5


def _wide(col, n):
    reps = n // 128
    if reps == 1:
        return col
    return jnp.concatenate([col] * reps, axis=1)


def _fold(a):
    n = a.shape[1] // 128
    acc = a[:, 0:128]
    for t in range(1, n):
        acc = acc + a[:, t * 128:(t + 1) * 128]
    return acc


def _kernel(x_hbm, wq_hbm, wkT_ref, wvT_ref, wo_hbm, w1T_hbm, w2_hbm, c_ref, wmod_hbm, g_ref,
            out_ref, dx_hbm, dwq_hbm, dwkT_ref, dwvT_ref, dwo_hbm, dw1T_hbm, dw2_hbm, dc_ref, dwmod_hbm,
            sx, swq, swo, sw12, swm, sems,
            xT, st1, h1T, modc, wqT, woT, wT12, wkv,
            Kaug, Vaug, KT, VT, Qs, QB, dOs, OT, dQT, SA, SB, mA, mB, P, linv_s, dKT, dVT,
            aW1, aW2, aWq, aWo, macc, dx2T, dh1T, h2s, dfs, facc, hacc, zs, WB, dQs, dscs, ACC, DS, DQ):
    i = pl.program_id(0)
    sw1 = sw12.at[0]
    sw2 = sw12.at[1]

    in_pairs = [(wmod_hbm, swm), (x_hbm, sx), (wq_hbm, swq), (wo_hbm, swo),
                (w1T_hbm, sw1), (w2_hbm, sw2)]

    def in_copy(k):
        return pltpu.make_async_copy(in_pairs[k][0], in_pairs[k][1], sems.at[k])

    out_pairs = [(swm, dwmod_hbm), (sx, dx_hbm), (swq, dwq_hbm), (swo, dwo_hbm),
                 (sw1, dw1T_hbm), (sw2, dw2_hbm)]

    def out_copy(k):
        return pltpu.make_async_copy(out_pairs[k][0], out_pairs[k][1], sems.at[6 + k])

    def transpose_into(dst, src_ref, ncols):
        nrows = src_ref.shape[0]

        def body(k, carry):
            c0 = pl.multiple_of(k * 128, 128)
            r0 = pl.multiple_of(k * 64, 64)
            dst[pl.ds(r0, 64), 0:nrows] = _pk(_dot_nt(_eye(128), src_ref[:, pl.ds(c0, 128)]).astype(BF16))
            return carry

        jax.lax.fori_loop(0, ncols // 128, body, 0)

    def repack_into(dst, src_ref, nrows):
        def body(k, carry):
            r0 = pl.multiple_of(k * 64, 64)
            q0 = pl.multiple_of(k * 32, 32)
            dst[pl.ds(q0, 32), :] = _pk(src_ref[pl.ds(r0, 64), :])
            return carry

        jax.lax.fori_loop(0, nrows // 64, body, 0)

    def zero_rows(ref, blk):
        def body(k, carry):
            r0 = pl.multiple_of(k * blk, blk)
            ref[pl.ds(r0, blk), :] = jnp.zeros((blk, ref.shape[1]), ref.dtype)
            return carry

        jax.lax.fori_loop(0, ref.shape[0] // blk, body, 0)

    def cast_rows(dst, src, nrows, blk):
        def body(k, carry):
            r0 = pl.multiple_of(k * blk, blk)
            dst[pl.ds(r0, blk), :] = src[pl.ds(r0, blk), :].astype(BF16)
            return carry

        jax.lax.fori_loop(0, nrows // blk, body, 0)

    def wmod_copy(part):
        lo, hi = (0, 2 * D) if part == 0 else (2 * D, 6 * D)
        return pltpu.make_async_copy(wmod_hbm.at[:, lo:hi], swm.at[:, lo:hi], sems.at[0 if part == 0 else 12])

    def dwmod_copy(part):
        lo, hi = (0, 2 * D) if part == 0 else (2 * D, 6 * D)
        return pltpu.make_async_copy(swm.at[:, lo:hi], dwmod_hbm.at[:, lo:hi], sems.at[6 if part == 0 else 7])

    def dx_copy(t):
        r0 = t * LW if isinstance(t, int) else pl.multiple_of(t * LW, LW)
        return pltpu.make_async_copy(sx.at[pl.ds(r0, LW), :], dx_hbm.at[pl.ds(r0, LW), :], sems.at[13 + t])

    def dmod_cols(k_lo, k_hi):
        cf = c_ref[...].astype(F32)
        sc = cf * _sigmoid(cf)
        scc = jnp.transpose(jnp.broadcast_to(sc, (128, D)))
        rid = jax.lax.broadcasted_iota(jnp.int32, (16, D), 0)

        def body(k, carry):
            c0 = pl.multiple_of(k * D, 128)
            row = jnp.sum(jnp.transpose(macc[k]), axis=0, keepdims=True)
            hi = row.astype(BF16).astype(F32)
            lo = row - hi
            lhs = jnp.where(rid == 0, hi, jnp.where(rid == 1, lo, 0.0)).astype(BF16)
            d2 = _dot_nt(lhs, swm[:, pl.ds(c0, D)])
            swm[:, pl.ds(c0, D)] = (_wide(scc, D) * row).astype(BF16)
            dscs[0:1, :] += d2[0:1] + d2[1:2]
            return carry

        jax.lax.fori_loop(k_lo, k_hi, body, 0)

    def mod_col(k):
        cf = c_ref[...].astype(F32)
        sc = cf * _sigmoid(cf)
        scb = jnp.broadcast_to(sc, (16, D)).astype(BF16)
        c0 = k * D if isinstance(k, int) else pl.multiple_of(k * D, 128)
        row = _dot(scb, swm[:, pl.ds(c0, D)])[0:1]
        row = row + jnp.where(jnp.logical_or(k == 1, k == 4), 1.0, 0.0)
        modc[k] = jnp.transpose(jnp.broadcast_to(row, (128, D)))

    def mod_cols(k_lo, k_hi):
        def body(k, carry):
            mod_col(k)
            return carry

        jax.lax.fori_loop(k_lo, k_hi, body, 0)

    def score_pass(n, Snext, mnext, c, m8):
        c0 = c * CKF
        z = pl.multiple_of(zs[0], 8)
        qT = _ld(QB[n])
        s = _dot(_ld(Kaug[c0 // 2:(c0 + CKF) // 2, :]), qT)
        Snext[pl.ds(z + c0, CKF), :] = s
        mc = jnp.max(s.reshape(CKF // 8, 8, VQ), axis=0)
        return mc if m8 is None else jnp.maximum(m8, mc)

    @pl.when(i == 0)
    @jax.named_scope('prologue')
    def _prologue():
        in_copy(1).start()
        wmod_copy(0).start()
        in_copy(2).start()
        in_copy(4).start()
        in_copy(5).start()
        in_copy(3).start()
        wmod_copy(1).start()
        zs[0] = 0

        macc[...] = jnp.zeros_like(macc)
        dKT[...] = jnp.zeros_like(dKT)
        dVT[...] = jnp.zeros_like(dVT)
        zero_rows(aW1, 64)
        zero_rows(aW2, 64)
        zero_rows(aWq, 64)
        zero_rows(aWo, 64)
        dQs[...] = jnp.zeros_like(dQs)
        dscs[...] = jnp.zeros_like(dscs)
        Qs[D:D + 16, :] = jnp.zeros((16, TQ), F32)

        z12 = jnp.zeros((HD - DH, D), F32)
        wkvT = jnp.concatenate([wkT_ref[...].astype(F32), z12, wvT_ref[...].astype(F32), z12],
                               axis=0).astype(BF16)
        eye128 = _eye(128)
        for c0 in range(0, D, 128):
            wkv[c0 // 2:(c0 + 128) // 2, :] = _pk(_dot_nt(eye128, wkvT[:, c0:c0 + 128]).astype(BF16))

        wmod_copy(0).wait()
        mod_cols(0, 2)
        in_copy(2).wait()
        transpose_into(wqT, swq, D)
        in_copy(1).wait()

        rowid = jax.lax.broadcasted_iota(jnp.int32, (HD, TQ), 0)
        ones_rows = jnp.logical_and(rowid >= DH, rowid < DH + 2)

        def ln1_block(t):
            t0 = pl.multiple_of(t * TQ, TQ)
            xt = jnp.transpose(sx[pl.ds(t0, TQ), :].astype(F32))
            xT[:, pl.ds(t0, TQ)] = _pk(xt.astype(BF16))
            mu = jnp.mean(xt, axis=0, keepdims=True)
            xc = xt - mu
            var = jnp.mean(xc * xc, axis=0, keepdims=True)
            rstd = jax.lax.rsqrt(var + EPS)
            st1[0:1, pl.ds(t0, TQ)] = mu
            st1[1:2, pl.ds(t0, TQ)] = rstd
            h1 = (xc * rstd * _wide(modc[1], TQ) + _wide(modc[0], TQ)).astype(BF16)
            h1T[:, pl.ds(t0, TQ)] = _pk(h1)
            kv = _dot(wkvT, h1)
            kt = kv[0:HD].astype(BF16)
            vt = jnp.where(ones_rows, 1.0, kv[HD:2 * HD]).astype(BF16)
            KT[:, pl.ds(t0, TQ)] = _pk(kt)
            VT[:, pl.ds(t0, TQ)] = _pk(vt)
            for k in range(TQ // 128):
                r0 = pl.multiple_of(t * (TQ // 2) + 64 * k, 64)
                Kaug[pl.ds(r0, 64), :] = _pk(_dot_nt(eye128, kt[:, 128 * k:128 * (k + 1)]).astype(BF16))
                Vaug[pl.ds(r0, 64), :] = _pk(_dot_nt(eye128, vt[:, 128 * k:128 * (k + 1)]).astype(BF16))

        def q_block(b):
            t0 = pl.multiple_of(b * TQ, TQ)
            Qs[0:D, :] = _dot(_ld(wqT[...]), _ld(h1T[:, pl.ds(t0, TQ)])) * (SCALE * LOG2E)
            for g in range(NG):
                qblk = Qs[g * GR:g * GR + GR + 16, :]
                qT = jnp.concatenate([qblk[0:HD], qblk[DH:DH + HD]], axis=1).astype(BF16)
                QB[b * NG + g] = _pk(qT)

        ln1_block(zs[0])

        def pq_body(b, carry):
            q_block(b)
            ln1_block(jnp.minimum(b + 1, NB - 1))
            return carry

        NW = 2 * NFC
        jax.lax.fori_loop(0, NB - NW, pq_body, 0)

        in_copy(4).wait()

        def pq2_body(b, carry):
            k = b - (NB - NW)

            @pl.when(k == NFC)
            def _():
                in_copy(5).wait()

            q_block(b)
            ln1_block(jnp.minimum(b + 1, NB - 1))
            r0 = pl.multiple_of((k % NFC) * FC, 32)
            for c0 in range(0, D, 128):
                wT12[k, c0 // 2:(c0 + 128) // 2, :] = _pk(
                    jnp.transpose(sw12[k // NFC, pl.ds(r0, FC), c0:c0 + 128]))
            return carry

        jax.lax.fori_loop(NB - NW, NB, pq2_body, 0)

        in_copy(3).wait()
        wmod_copy(1).wait()
        for c0 in range(0, D, 128):
            woT[c0 // 2:(c0 + 128) // 2, :] = _pk(jnp.transpose(swo[:, c0:c0 + 128]))
        for k in range(2, 6):
            mod_col(k)
        m8 = None
        for c in range(S // CKF):
            m8 = score_pass(0, SA, mA, c, m8)
        mA[...] = m8


    t0 = pl.multiple_of(i * TQ, TQ)

    def fwd_step(g, n, Scur, mcur, Snext, mnext):
        m = jnp.max(mcur[...], axis=0, keepdims=True)
        z = pl.multiple_of(zs[0], 8)
        m8 = None
        acc = None
        nch = S // CKF
        for cc in range(nch + SKEW):
            if cc < nch:
                m8 = score_pass(n, Snext, mnext, cc, m8)
            if cc >= SKEW:
                c0 = (cc - SKEW) * CKF
                p = jnp.exp2(Scur[pl.ds(z + c0, CKF), :] - m).astype(BF16)
                P[g, c0 // 2:(c0 + CKF) // 2, :] = _pk(p)
                r = _dot(_ld(VT[:, c0:c0 + CKF]), p)
                acc = r if acc is None else acc + r
        mnext[...] = m8
        ACC[g] = acc[0:24, :]

    def fwd_body(gg, carry):
        g = UF * gg
        n = i * NG + g
        for u in range(0, UF, 2):
            fwd_step(g + u, n + u + 1, SA, mA, SB, mB)
            fwd_step(g + u + 1, jnp.minimum(n + u + 2, NB * NG - 1), SB, mB, SA, mA)
        return carry

    with jax.named_scope('fwdloop'):
        jax.lax.fori_loop(0, NG // UF, fwd_body, 0)

    with jax.named_scope('mid1'):
        ga = _wide(modc[2], TQ)
        sb = _wide(modc[3], TQ)
        cb1 = _wide(modc[4], TQ)
        gb = _wide(modc[5], TQ)
        eye128 = _eye(128)

        gT = jnp.transpose(g_ref[...].astype(F32))
        dfs[...] = _pk((gT * gb).astype(BF16))

        for g in range(NG):
            acc = ACC[g]
            linv = 1.0 / acc[DH:DH + 1, :]
            linv_s[g] = jnp.broadcast_to(linv, (8, VQ))
            o = acc[0:DH, :] * linv
            OT[g * GR:(g + 1) * GR, :] = jnp.concatenate([o[:, 0:TQ], o[:, TQ:VQ]], axis=0)
        tp = pl.multiple_of(jnp.maximum(i - 1, 0) * TQ, TQ)
        h1p = _ld(h1T[:, pl.ds(tp, TQ)])
        dQp = _ld(dQs[...])
        aWq[0:256, :] += _dot_nt(h1p[0:256], dQp)
        OTb = OT[...].astype(BF16)
        attn = _dot(_ld(woT[...]), OTb)
        aWq[256:D, :] += _dot_nt(h1p[256:D], dQp)
        x2 = _ld(xT[:, pl.ds(t0, TQ)]).astype(F32) + ga * attn
        mu2 = jnp.mean(x2, axis=0, keepdims=True)
        xc2 = x2 - mu2
        var2 = jnp.mean(xc2 * xc2, axis=0, keepdims=True)
        rstd2 = jax.lax.rsqrt(var2 + EPS)
        xh2 = xc2 * rstd2
        h2s[...] = _pk((xh2 * cb1 + sb).astype(BF16))

    def ffn_body(j, carry):
        h2 = _ld(h2s[...])
        df = _ld(dfs[...])
        a_parts = []
        du_parts = []
        for sb_ in range(FC // FS):
            f0 = pl.multiple_of(j * FC + sb_ * FS, 32)
            u = _dot(sw1[pl.ds(f0, FS), :], h2)
            da = _dot(sw2[pl.ds(f0, FS), :], df)
            sg = _sigmoid(u)
            a = (u * sg).astype(BF16)
            du = (da * (sg * (1.0 + u * (1.0 - sg)))).astype(BF16)
            aW2[pl.ds(f0, FS), :] += _dot_nt(a, df)
            aW1[pl.ds(f0, FS), :] += _dot_nt(du, h2)
            a_parts.append(a)
            du_parts.append(du)
        a = jnp.concatenate(a_parts, axis=0)
        du = jnp.concatenate(du_parts, axis=0)
        facc[...] = jnp.where(j > 0, facc[...], 0.0) + _dot(_ld(wT12[NFC + j]), a)
        hacc[...] = jnp.where(j > 0, hacc[...], 0.0) + _dot(_ld(wT12[j]), du)
        return carry

    with jax.named_scope('ffnloop'):
        jax.lax.fori_loop(0, NFC, ffn_body, 0)

    with jax.named_scope('mid2'):
        dh1T[:, pl.ds(tp, TQ)] = _dot(swq[...], _ld(dQs[...]))
        f = facc[...]
        outT = (x2 + gb * f).astype(BF16)
        out_ref[...] = jnp.transpose(outT)
        macc[5] += _fold(gT * f)
        dh2 = hacc[...]
        macc[4] += _fold(dh2 * xh2)
        macc[3] += _fold(dh2)
        dxh = dh2 * cb1
        m1 = jnp.mean(dxh, axis=0, keepdims=True)
        m2 = jnp.mean(dxh * xh2, axis=0, keepdims=True)
        dx2 = gT + rstd2 * (dxh - m1 - xh2 * m2)
        dx2T[:, pl.ds(t0, TQ)] = dx2
        macc[2] += _fold(dx2 * attn)
        dattn = (dx2 * ga).astype(BF16)
        dOs[...] = _dot(swo[...], dattn)
        aWo[...] += _dot_nt(OTb, dattn)
        for g in range(NG):
            dob = dOs[g * GR:(g + 1) * GR, :]
            ob = OT[g * GR:(g + 1) * GR, :]
            do = jnp.concatenate([dob[0:DH], dob[DH:GR]], axis=1)
            o = jnp.concatenate([ob[0:DH], ob[DH:GR]], axis=1)
            linv = linv_s[g][0:1, :]
            nd = -jnp.sum(do * o, axis=0, keepdims=True) * linv
            nd_hi = nd.astype(BF16).astype(F32)
            nd_lo = nd - nd_hi
            W = jnp.concatenate([do * linv, nd_hi, nd_lo, jnp.zeros((HD - DH - 2, VQ), F32)],
                                axis=0).astype(BF16)
            WB[g] = _pk(W)
        DS[...] = jnp.zeros_like(DS)
        DQ[...] = jnp.zeros_like(DQ)

    @pl.when(i == NB - 1)
    @jax.named_scope('earlyout')
    def _early_out():
        cast_rows(swo, aWo, D, 64)
        cast_rows(sw1, aW1, FF, 64)
        cast_rows(sw2, aW2, FF, 64)
        out_copy(3).start()
        out_copy(4).start()
        out_copy(5).start()
        dmod_cols(2, 6)
        dwmod_copy(1).start()

    def finish_dq(g, dq):
        dq = dq[0:DH, :] * SCALE
        r0 = g * GR if isinstance(g, int) else pl.multiple_of(g * GR, 8)
        dQT[pl.ds(r0, GR), :] = jnp.concatenate([dq[:, 0:TQ], dq[:, TQ:VQ]], axis=0)

    def bwd_body(gg, carry):
        gs = [gg * UB + u for u in range(UB)]
        gp = jnp.maximum(gs[0] - 1, 0)
        qTs = [_ld(QB[i * NG + g]) for g in gs]
        Ws = [_ld(WB[g]) for g in gs]
        nch = S // CKB
        H2 = CKB // 2
        dq = DQ[...]
        prev = (gp, _ld(QB[i * NG + gp]), S - CKB, _ld(DS[...]))
        for u in range(UB):
            for c in range(nch):
                c0 = c * CKB
                pg, pq, pc0, pds = prev
                dpa = _dot(_ld(Vaug[c0 // 2:(c0 + H2) // 2, :]), Ws[u])
                dKT[:, pc0:pc0 + CKB] += _dot_nt(pq, pds)
                dpb = _dot(_ld(Vaug[(c0 + H2) // 2:(c0 + CKB) // 2, :]), Ws[u])
                p = _ld(P[gs[u], c0 // 2:(c0 + CKB) // 2, :])
                dVT[:, c0:c0 + CKB] += _dot_nt(Ws[u], p)
                r = _dot(_ld(KT[:, pc0:pc0 + CKB]), pds)
                dq = r if dq is None else dq + r
                if pc0 + CKB == S:
                    finish_dq(pg, dq)
                    dq = None
                pf = p.astype(F32)
                ds = jnp.concatenate([(pf[:H2] * dpa).astype(BF16), (pf[H2:] * dpb).astype(BF16)], axis=0)
                prev = (gs[u], qTs[u], c0, ds)
        DS[...] = _pk(prev[3])
        DQ[...] = dq
        return carry

    with jax.named_scope('bwdloop'):
        jax.lax.fori_loop(0, NG // UB, bwd_body, 0)

    with jax.named_scope('post'):
        pds = _ld(DS[...])
        dKT[:, S - CKB:S] += _dot_nt(_ld(QB[i * NG + NG - 1]), pds)
        finish_dq(NG - 1, DQ[...] + _dot(_ld(KT[:, S - CKB:S]), pds))
        dQs[...] = _pk(dQT[...].astype(BF16))

    @pl.when(i == NB - 1)
    @jax.named_scope('epilogue')
    def _epilogue():
        dQb = _ld(dQs[...])
        dh1T[:, S - TQ:S] = _dot(swq[...], dQb)
        swq[...] = (aWq[...] + _dot_nt(_ld(h1T[:, S - TQ:S]), dQb)).astype(BF16)
        out_copy(2).start()
        dkv = jnp.concatenate([dKT[...] * (1.0 / LOG2E), dVT[...]], axis=0).astype(BF16)
        dwkvT = _dot_nt(dkv, _ld(h1T[...]))
        dwkT_ref[...] = dwkvT[0:DH].astype(BF16)
        dwvT_ref[...] = dwkvT[HD:HD + DH].astype(BF16)
        KT[...] = _pk(dkv[0:HD])
        VT[...] = _pk(dkv[HD:2 * HD])
        ca1 = modc[1]
        eye = _eye(128)

        def ln1b_body(t, carry):
            c0 = pl.multiple_of(t * LW, LW)
            dkvc = jnp.concatenate([_ld(KT[:, pl.ds(c0, LW)]), _ld(VT[:, pl.ds(c0, LW)])], axis=0)
            dh1 = dh1T[:, pl.ds(c0, LW)] + _dot(_ld(wkv[...]), dkvc)
            mu = st1[0:1, pl.ds(c0, LW)]
            rstd = st1[1:2, pl.ds(c0, LW)]
            xh = (_ld(xT[:, pl.ds(c0, LW)]).astype(F32) - mu) * rstd
            macc[1] += _fold(dh1 * xh)
            macc[0] += _fold(dh1)
            dxh1 = dh1 * _wide(ca1, LW)
            n1 = jnp.mean(dxh1, axis=0, keepdims=True)
            n2 = jnp.mean(dxh1 * xh, axis=0, keepdims=True)
            dxt = (dx2T[:, pl.ds(c0, LW)] + rstd * (dxh1 - n1 - xh * n2)).astype(BF16)
            for k in range(LW // 128):
                r0 = pl.multiple_of(t * LW + 128 * k, 128)
                sx[pl.ds(r0, 128), :] = _dot_nt(eye, dxt[:, 128 * k:128 * (k + 1)]).astype(BF16)
            dx_copy(t).start()
            return carry

        jax.lax.fori_loop(0, S // LW, ln1b_body, 0)

        dmod_cols(0, 2)
        dwmod_copy(0).start()
        cf = c_ref[...].astype(F32)
        sgc = _sigmoid(cf)
        dc_ref[...] = (dscs[0:1, :] * (sgc * (1.0 + cf * (1.0 - sgc)))).astype(BF16)
        dwmod_copy(0).wait()
        dwmod_copy(1).wait()
        for t in range(S // LW):
            dx_copy(t).wait()
        for k in range(2, 6):
            out_copy(k).wait()


@jax.jit
def pallas_adaLN_cond__grouped_kv_mqa__dense_activation_silu__prompt_kernel(
    A_x: jax.Array,
    A_wq: jax.Array,
    A_wk: jax.Array,
    A_wv: jax.Array,
    A_wo: jax.Array,
    B_x: jax.Array,
    B_w1: jax.Array,
    B_w2: jax.Array,
    c: jax.Array,
    w_mod: jax.Array,
    grad_out: jax.Array,
):
    x = A_x.reshape(S, D)
    g = grad_out.reshape(S, D)

    def full(shape):
        return pl.BlockSpec(shape, lambda i: (0,) * len(shape))

    hbm = pl.BlockSpec(memory_space=pl.ANY)

    in_specs = [
        hbm, hbm, full((DH, D)), full((DH, D)), hbm,
        hbm, hbm, full((1, D)), hbm,
        pl.BlockSpec((TQ, D), lambda i: (i, 0)),
    ]
    out_specs = [
        pl.BlockSpec((TQ, D), lambda i: (i, 0)),
        hbm, hbm, full((DH, D)), full((DH, D)), hbm,
        hbm, hbm, full((1, D)), hbm,
    ]
    out_shape = [
        jax.ShapeDtypeStruct((S, D), BF16), jax.ShapeDtypeStruct((S, D), BF16),
        jax.ShapeDtypeStruct((D, D), BF16), jax.ShapeDtypeStruct((DH, D), BF16),
        jax.ShapeDtypeStruct((DH, D), BF16), jax.ShapeDtypeStruct((D, D), BF16),
        jax.ShapeDtypeStruct((FF, D), BF16), jax.ShapeDtypeStruct((FF, D), BF16),
        jax.ShapeDtypeStruct((1, D), BF16), jax.ShapeDtypeStruct((D, 6 * D), BF16),
    ]
    scratch = [
        pltpu.VMEM((S, D), BF16),
        pltpu.VMEM((D, D), BF16),
        pltpu.VMEM((D, D), BF16),
        pltpu.VMEM((2, FF, D), BF16),
        pltpu.VMEM((D, 6 * D), BF16),
        pltpu.SemaphoreType.DMA((13 + S // LW,)),
        pltpu.VMEM((D // 2, S), U32),
        pltpu.VMEM((8, S), F32),
        pltpu.VMEM((D // 2, S), U32),
        pltpu.VMEM((6, D, 128), F32),
        pltpu.VMEM((D // 2, D), U32),
        pltpu.VMEM((D // 2, D), U32),
        pltpu.VMEM((2 * NFC, D // 2, FC), U32),
        pltpu.VMEM((D // 2, 2 * HD), U32),
        pltpu.VMEM((S // 2, HD), U32),
        pltpu.VMEM((S // 2, HD), U32),
        pltpu.VMEM((HD // 2, S), U32),
        pltpu.VMEM((HD // 2, S), U32),
        pltpu.VMEM((D + 16, TQ), F32),
        pltpu.VMEM((NB * NG, HD // 2, VQ), U32),
        pltpu.VMEM((D, TQ), F32),
        pltpu.VMEM((D, TQ), F32),
        pltpu.VMEM((D, TQ), F32),
        pltpu.VMEM((S, VQ), F32),
        pltpu.VMEM((S, VQ), F32),
        pltpu.VMEM((8, VQ), F32),
        pltpu.VMEM((8, VQ), F32),
        pltpu.VMEM((NG, S // 2, VQ), U32),
        pltpu.VMEM((NG, 8, VQ), F32),
        pltpu.VMEM((HD, S), F32),
        pltpu.VMEM((HD, S), F32),
        pltpu.VMEM((FF, D), F32),
        pltpu.VMEM((FF, D), F32),
        pltpu.VMEM((D, D), F32),
        pltpu.VMEM((D, D), F32),
        pltpu.VMEM((6, D, 128), F32),
        pltpu.VMEM((D, S), F32),
        pltpu.VMEM((D, S), F32),
        pltpu.VMEM((D // 2, TQ), U32),
        pltpu.VMEM((D // 2, TQ), U32),
        pltpu.VMEM((D, TQ), F32),
        pltpu.VMEM((D, TQ), F32),
        pltpu.SMEM((1,), jnp.int32),
        pltpu.VMEM((NG, HD // 2, VQ), U32),
        pltpu.VMEM((D // 2, TQ), U32),
        pltpu.VMEM((8, D), F32),
        pltpu.VMEM((NG, 24, VQ), F32),
        pltpu.VMEM((CKB // 2, VQ), U32),
        pltpu.VMEM((HD, VQ), F32),
    ]
    outs = pl.pallas_call(
        _kernel,
        grid=(NB,),
        in_specs=in_specs,
        out_specs=out_specs,
        out_shape=out_shape,
        scratch_shapes=scratch,
        compiler_params=pltpu.CompilerParams(
            dimension_semantics=("arbitrary",),
            vmem_limit_bytes=126 * 1024 * 1024,
        ),
    )(x, A_wq, A_wk.T, A_wv.T, A_wo, B_w1.T, B_w2, c, w_mod, g)
    out, dx, dwq, dwkT, dwvT, dwo, dw1T, dw2, dc, dwmod = outs
    return (out.reshape(1, S, D), dx.reshape(1, S, D), dwq, dwkT.T, dwvT.T, dwo, dw1T.T, dw2, dc, dwmod)
```

```python
import jax
import jax.numpy as jnp
import jax.experimental.pallas as pl
import jax.experimental.pallas.tpu as pltpu

F32 = jnp.float32
BF16 = jnp.bfloat16
U32 = jnp.uint32

S = 2048
D = 640
H = 32
DH = 20
FF = 1728
FC = 864
NFC = FF // FC
FS = 288
EPS = 1e-5

TQ = 256
NB = S // TQ
HP = 2
NG = H // HP
GR = HP * DH
VQ = HP * TQ
CKF = 128
CKB = 256
HD = 32
UF = 2
UB = 4
SKEW = 1
LW = 512

LOG2E = 1.4426950408889634
SCALE = DH ** (-0.5)

_NT = (((1,), (1,)), ((), ()))


def _dot(a, b):
    return jnp.dot(a, b, preferred_element_type=F32)


def _dot_nt(a, b):
    return jax.lax.dot_general(a, b, _NT, preferred_element_type=F32)


def _ld(v):
    return pltpu.bitcast(v, BF16)


def _pk(v):
    return pltpu.bitcast(v, U32)


def _eye(n, dtype=BF16):
    r = jax.lax.broadcasted_iota(jnp.int32, (n, n), 0)
    c = jax.lax.broadcasted_iota(jnp.int32, (n, n), 1)
    return jnp.where(r == c, 1.0, 0.0).astype(dtype)


def _sigmoid(x):
    return 0.5 * jnp.tanh(0.5 * x) + 0.5


def _wide(col, n):
    reps = n // 128
    if reps == 1:
        return col
    return jnp.concatenate([col] * reps, axis=1)


def _fold(a):
    n = a.shape[1] // 128
    acc = a[:, 0:128]
    for t in range(1, n):
        acc = acc + a[:, t * 128:(t + 1) * 128]
    return acc


def _kernel(x_hbm, wq_hbm, wkT_ref, wvT_ref, wo_hbm, w1T_hbm, w2_hbm, c_ref, wmod_hbm, g_ref,
            out_ref, dx_hbm, dwq_hbm, dwkT_ref, dwvT_ref, dwo_hbm, dw1T_hbm, dw2_hbm, dc_ref, dwmod_hbm,
            sx, swq, swo, sw12, swm, sems,
            xT, st1, h1T, modc, wqT, woT, wT12, wkv,
            Kaug, Vaug, KT, VT, Qs, QB, dOs, OT, dQT, SA, SB, mA, mB, P, linv_s, dKT, dVT,
            aW1, aW2, aWq, aWo, macc, dx2T, dh1T, h2s, dfs, facc, hacc, zs, WB, dQs, dscs, ACC, DS, DQ, akv):
    i = pl.program_id(0)
    sw1 = sw12.at[0]
    sw2 = sw12.at[1]

    in_pairs = [(wmod_hbm, swm), (x_hbm, sx), (wq_hbm, swq), (wo_hbm, swo),
                (w1T_hbm, sw1), (w2_hbm, sw2)]

    def in_copy(k):
        return pltpu.make_async_copy(in_pairs[k][0], in_pairs[k][1], sems.at[k])

    out_pairs = [(swm, dwmod_hbm), (sx, dx_hbm), (swq, dwq_hbm), (swo, dwo_hbm),
                 (sw1, dw1T_hbm), (sw2, dw2_hbm)]

    def out_copy(k):
        return pltpu.make_async_copy(out_pairs[k][0], out_pairs[k][1], sems.at[6 + k])

    def transpose_into(dst, src_ref, ncols):
        nrows = src_ref.shape[0]

        def body(k, carry):
            c0 = pl.multiple_of(k * 128, 128)
            r0 = pl.multiple_of(k * 64, 64)
            dst[pl.ds(r0, 64), 0:nrows] = _pk(_dot_nt(_eye(128), src_ref[:, pl.ds(c0, 128)]).astype(BF16))
            return carry

        jax.lax.fori_loop(0, ncols // 128, body, 0)

    def cast_rows(dst, src, nrows, blk):
        def body(k, carry):
            r0 = pl.multiple_of(k * blk, blk)
            dst[pl.ds(r0, blk), :] = src[pl.ds(r0, blk), :].astype(BF16)
            return carry

        jax.lax.fori_loop(0, nrows // blk, body, 0)

    def wmod_copy(part):
        lo, hi = (0, 2 * D) if part == 0 else (2 * D, 6 * D)
        return pltpu.make_async_copy(wmod_hbm.at[:, lo:hi], swm.at[:, lo:hi], sems.at[0 if part == 0 else 12])

    def dwmod_copy(k):
        c0 = k * D if isinstance(k, int) else pl.multiple_of(k * D, 128)
        return pltpu.make_async_copy(swm.at[:, pl.ds(c0, D)], dwmod_hbm.at[:, pl.ds(c0, D)],
                                     sems.at[13 + S // LW + k])

    def x_copy(b):
        r0 = b * TQ if isinstance(b, int) else pl.multiple_of(b * TQ, TQ)
        return pltpu.make_async_copy(x_hbm.at[pl.ds(r0, TQ), :], sx.at[pl.ds(r0, TQ), :],
                                     sems.at[13 + S // LW + 6 + b])

    def dwq_copy(t):
        QR = D // (S // LW)
        r0 = t * QR if isinstance(t, int) else pl.multiple_of(t * QR, 16)
        return pltpu.make_async_copy(swq.at[pl.ds(r0, QR), :], dwq_hbm.at[pl.ds(r0, QR), :],
                                     sems.at[13 + S // LW + 6 + NB + t])

    def dx_copy(t):
        r0 = t * LW if isinstance(t, int) else pl.multiple_of(t * LW, LW)
        return pltpu.make_async_copy(sx.at[pl.ds(r0, LW), :], dx_hbm.at[pl.ds(r0, LW), :], sems.at[13 + t])

    def dmod_cols(k_lo, k_hi):
        cf = c_ref[...].astype(F32)
        sc = cf * _sigmoid(cf)
        scc = jnp.transpose(jnp.broadcast_to(sc, (128, D)))
        rid = jax.lax.broadcasted_iota(jnp.int32, (16, D), 0)

        def body(k, carry):
            c0 = pl.multiple_of(k * D, 128)
            row = jnp.sum(jnp.transpose(macc[k]), axis=0, keepdims=True)
            hi = row.astype(BF16).astype(F32)
            lo = row - hi
            lhs = jnp.where(rid == 0, hi, jnp.where(rid == 1, lo, 0.0)).astype(BF16)
            d2 = _dot_nt(lhs, swm[:, pl.ds(c0, D)])
            swm[:, pl.ds(c0, D)] = (_wide(scc, D) * row).astype(BF16)
            dscs[0:1, :] += d2[0:1] + d2[1:2]
            dwmod_copy(k).start()
            return carry

        jax.lax.fori_loop(k_lo, k_hi, body, 0)

    def mod_col(k):
        cf = c_ref[...].astype(F32)
        sc = cf * _sigmoid(cf)
        scb = jnp.broadcast_to(sc, (16, D)).astype(BF16)
        c0 = k * D if isinstance(k, int) else pl.multiple_of(k * D, 128)
        row = _dot(scb, swm[:, pl.ds(c0, D)])[0:1]
        row = row + jnp.where(jnp.logical_or(k == 1, k == 4), 1.0, 0.0)
        modc[k] = jnp.transpose(jnp.broadcast_to(row, (128, D)))

    def mod_cols(k_lo, k_hi):
        def body(k, carry):
            mod_col(k)
            return carry

        jax.lax.fori_loop(k_lo, k_hi, body, 0)

    def score_pass(n, Snext, mnext, c, m8):
        c0 = c * CKF
        z = pl.multiple_of(zs[0], 8)
        qT = _ld(QB[n])
        s = _dot(_ld(Kaug[c0 // 2:(c0 + CKF) // 2, :]), qT)
        Snext[pl.ds(z + c0, CKF), :] = s
        mc = jnp.max(s.reshape(CKF // 8, 8, VQ), axis=0)
        return mc if m8 is None else jnp.maximum(m8, mc)

    @pl.when(i == 0)
    @jax.named_scope('prologue')
    def _prologue():
        wmod_copy(0).start()
        x_copy(0).start()
        in_copy(2).start()
        for b in range(1, NB):
            x_copy(b).start()
        zs[0] = 0

        macc[...] = jnp.zeros_like(macc)
        dKT[...] = jnp.zeros_like(dKT)
        dVT[...] = jnp.zeros_like(dVT)
        dQs[...] = jnp.zeros_like(dQs)
        dscs[...] = jnp.zeros_like(dscs)
        Qs[D:D + 16, :] = jnp.zeros((16, TQ), F32)

        z12 = jnp.zeros((HD - DH, D), F32)
        wkvT = jnp.concatenate([wkT_ref[...].astype(F32), z12, wvT_ref[...].astype(F32), z12],
                               axis=0).astype(BF16)
        eye128 = _eye(128)
        for c0 in range(0, D, 128):
            wkv[c0 // 2:(c0 + 128) // 2, :] = _pk(_dot_nt(eye128, wkvT[:, c0:c0 + 128]).astype(BF16))

        wmod_copy(0).wait()
        mod_cols(0, 2)

        rowid = jax.lax.broadcasted_iota(jnp.int32, (HD, TQ), 0)
        ones_rows = jnp.logical_and(rowid >= DH, rowid < DH + 2)

        def ln1_block(t):
            t0 = pl.multiple_of(t * TQ, TQ)
            xt = jnp.transpose(sx[pl.ds(t0, TQ), :].astype(F32))
            xT[:, pl.ds(t0, TQ)] = _pk(xt.astype(BF16))
            mu = jnp.mean(xt, axis=0, keepdims=True)
            xc = xt - mu
            var = jnp.mean(xc * xc, axis=0, keepdims=True)
            rstd = jax.lax.rsqrt(var + EPS)
            st1[0:1, pl.ds(t0, TQ)] = mu
            st1[1:2, pl.ds(t0, TQ)] = rstd
            h1 = (xc * rstd * _wide(modc[1], TQ) + _wide(modc[0], TQ)).astype(BF16)
            h1T[:, pl.ds(t0, TQ)] = _pk(h1)
            kv = _dot(wkvT, h1)
            kt = kv[0:HD].astype(BF16)
            vt = jnp.where(ones_rows, 1.0, kv[HD:2 * HD]).astype(BF16)
            KT[:, pl.ds(t0, TQ)] = _pk(kt)
            VT[:, pl.ds(t0, TQ)] = _pk(vt)
            for k in range(TQ // 128):
                r0 = pl.multiple_of(t * (TQ // 2) + 64 * k, 64)
                Kaug[pl.ds(r0, 64), :] = _pk(_dot_nt(eye128, kt[:, 128 * k:128 * (k + 1)]).astype(BF16))
                Vaug[pl.ds(r0, 64), :] = _pk(_dot_nt(eye128, vt[:, 128 * k:128 * (k + 1)]).astype(BF16))

        def q_block(b):
            t0 = pl.multiple_of(b * TQ, TQ)
            Qs[0:D, :] = _dot(_ld(wqT[...]), _ld(h1T[:, pl.ds(t0, TQ)])) * (SCALE * LOG2E)
            for g in range(NG):
                qblk = Qs[g * GR:g * GR + GR + 16, :]
                qT = jnp.concatenate([qblk[0:HD], qblk[DH:DH + HD]], axis=1).astype(BF16)
                QB[b * NG + g] = _pk(qT)

        x_copy(0).wait()
        ln1_block(zs[0])
        in_copy(2).wait()
        in_copy(4).start()
        in_copy(5).start()
        in_copy(3).start()
        wmod_copy(1).start()
        transpose_into(wqT, swq, D)

        def pq_body(b, carry):
            x_copy(b + 1).wait()
            q_block(b)
            ln1_block(jnp.minimum(b + 1, NB - 1))
            return carry

        NW = 2 * NFC
        jax.lax.fori_loop(0, NB - NW, pq_body, 0)

        in_copy(4).wait()

        def pq2_body(b, carry):
            k = b - (NB - NW)

            @pl.when(k == NFC)
            def _():
                in_copy(5).wait()

            @pl.when(b + 1 < NB)
            def _():
                x_copy(b + 1).wait()

            q_block(b)
            ln1_block(jnp.minimum(b + 1, NB - 1))
            r0 = pl.multiple_of((k % NFC) * FC, 32)
            for c0 in range(0, D, 128):
                wT12[k, c0 // 2:(c0 + 128) // 2, :] = _pk(
                    jnp.transpose(sw12[k // NFC, pl.ds(r0, FC), c0:c0 + 128]))
            return carry

        jax.lax.fori_loop(NB - NW, NB, pq2_body, 0)

        in_copy(3).wait()
        wmod_copy(1).wait()
        for c0 in range(0, D, 128):
            woT[c0 // 2:(c0 + 128) // 2, :] = _pk(jnp.transpose(swo[:, c0:c0 + 128]))
        for k in range(2, 6):
            mod_col(k)
        m8 = None
        for c in range(S // CKF):
            m8 = score_pass(0, SA, mA, c, m8)
        mA[...] = m8


    t0 = pl.multiple_of(i * TQ, TQ)

    def fwd_step(g, n, Scur, mcur, Snext, mnext):
        m = jnp.max(mcur[...], axis=0, keepdims=True)
        z = pl.multiple_of(zs[0], 8)
        m8 = None
        acc = None
        nch = S // CKF
        for cc in range(nch + SKEW):
            if cc < nch:
                m8 = score_pass(n, Snext, mnext, cc, m8)
            if cc >= SKEW:
                c0 = (cc - SKEW) * CKF
                p = jnp.exp2(Scur[pl.ds(z + c0, CKF), :] - m).astype(BF16)
                P[g, c0 // 2:(c0 + CKF) // 2, :] = _pk(p)
                r = _dot(_ld(VT[:, c0:c0 + CKF]), p)
                acc = r if acc is None else acc + r
        mnext[...] = m8
        ACC[g] = acc[0:24, :]

    def fwd_body(gg, carry):
        g = UF * gg
        n = i * NG + g
        for u in range(0, UF, 2):
            fwd_step(g + u, n + u + 1, SA, mA, SB, mB)
            fwd_step(g + u + 1, jnp.minimum(n + u + 2, NB * NG - 1), SB, mB, SA, mA)
        return carry

    with jax.named_scope('fwdloop'):
        jax.lax.fori_loop(0, NG // UF, fwd_body, 0)

    with jax.named_scope('mid1'):
        ga = _wide(modc[2], TQ)
        sb = _wide(modc[3], TQ)
        cb1 = _wide(modc[4], TQ)
        gb = _wide(modc[5], TQ)

        gT = jnp.transpose(g_ref[...].astype(F32))
        dfs[...] = _pk((gT * gb).astype(BF16))

        for g in range(NG):
            acc = ACC[g]
            linv = 1.0 / acc[DH:DH + 1, :]
            linv_s[g] = jnp.broadcast_to(linv, (8, VQ))
            o = acc[0:DH, :] * linv
            OT[g * GR:(g + 1) * GR, :] = jnp.concatenate([o[:, 0:TQ], o[:, TQ:VQ]], axis=0)
        tp = pl.multiple_of(jnp.maximum(i - 1, 0) * TQ, TQ)
        h1p = _ld(h1T[:, pl.ds(tp, TQ)])
        dQp = _ld(dQs[...])
        aWq[0:256, :] = jnp.where(i > 0, aWq[0:256, :], 0.0) + _dot_nt(h1p[0:256], dQp)
        OTb = OT[...].astype(BF16)
        attn = _dot(_ld(woT[...]), OTb)
        aWq[256:D, :] = jnp.where(i > 0, aWq[256:D, :], 0.0) + _dot_nt(h1p[256:D], dQp)
        x2 = _ld(xT[:, pl.ds(t0, TQ)]).astype(F32) + ga * attn
        mu2 = jnp.mean(x2, axis=0, keepdims=True)
        xc2 = x2 - mu2
        var2 = jnp.mean(xc2 * xc2, axis=0, keepdims=True)
        rstd2 = jax.lax.rsqrt(var2 + EPS)
        xh2 = xc2 * rstd2
        h2s[...] = _pk((xh2 * cb1 + sb).astype(BF16))

    def ffn_body(j, carry):
        h2 = _ld(h2s[...])
        df = _ld(dfs[...])
        a_parts = []
        du_parts = []
        for sb_ in range(FC // FS):
            f0 = pl.multiple_of(j * FC + sb_ * FS, 32)
            u = _dot(sw1[pl.ds(f0, FS), :], h2)
            da = _dot(sw2[pl.ds(f0, FS), :], df)
            sg = _sigmoid(u)
            a = (u * sg).astype(BF16)
            du = (da * (sg * (1.0 + u * (1.0 - sg)))).astype(BF16)
            aW2[pl.ds(f0, FS), :] = jnp.where(i > 0, aW2[pl.ds(f0, FS), :], 0.0) + _dot_nt(a, df)
            aW1[pl.ds(f0, FS), :] = jnp.where(i > 0, aW1[pl.ds(f0, FS), :], 0.0) + _dot_nt(du, h2)
            a_parts.append(a)
            du_parts.append(du)
        a = jnp.concatenate(a_parts, axis=0)
        du = jnp.concatenate(du_parts, axis=0)
        facc[...] = jnp.where(j > 0, facc[...], 0.0) + _dot(_ld(wT12[NFC + j]), a)
        hacc[...] = jnp.where(j > 0, hacc[...], 0.0) + _dot(_ld(wT12[j]), du)
        return carry

    with jax.named_scope('ffnloop'):
        jax.lax.fori_loop(0, NFC, ffn_body, 0)

    with jax.named_scope('mid2'):
        dh1T[:, pl.ds(tp, TQ)] = _dot(swq[...], _ld(dQs[...]))
        f = facc[...]
        outT = (x2 + gb * f).astype(BF16)
        out_ref[...] = jnp.transpose(outT)
        macc[5] += _fold(gT * f)
        dh2 = hacc[...]
        macc[4] += _fold(dh2 * xh2)
        macc[3] += _fold(dh2)
        dxh = dh2 * cb1
        m1 = jnp.mean(dxh, axis=0, keepdims=True)
        m2 = jnp.mean(dxh * xh2, axis=0, keepdims=True)
        dx2 = gT + rstd2 * (dxh - m1 - xh2 * m2)
        dx2T[:, pl.ds(t0, TQ)] = dx2
        macc[2] += _fold(dx2 * attn)
        dattn = (dx2 * ga).astype(BF16)
        dOs[...] = _dot(swo[...], dattn)
        aWo[...] = jnp.where(i > 0, aWo[...], 0.0) + _dot_nt(OTb, dattn)
        for g in range(NG):
            dob = dOs[g * GR:(g + 1) * GR, :]
            ob = OT[g * GR:(g + 1) * GR, :]
            do = jnp.concatenate([dob[0:DH], dob[DH:GR]], axis=1)
            o = jnp.concatenate([ob[0:DH], ob[DH:GR]], axis=1)
            linv = linv_s[g][0:1, :]
            nd = -jnp.sum(do * o, axis=0, keepdims=True) * linv
            nd_hi = nd.astype(BF16).astype(F32)
            nd_lo = nd - nd_hi
            W = jnp.concatenate([do * linv, nd_hi, nd_lo, jnp.zeros((HD - DH - 2, VQ), F32)],
                                axis=0).astype(BF16)
            WB[g] = _pk(W)
        DS[...] = jnp.zeros_like(DS)
        DQ[...] = jnp.zeros_like(DQ)

    @pl.when(i == NB - 1)
    @jax.named_scope('earlyout')
    def _early_out():
        cast_rows(swo, aWo, D, 64)
        cast_rows(sw1, aW1, FF, 64)
        cast_rows(sw2, aW2, FF, 64)
        out_copy(3).start()
        out_copy(4).start()
        out_copy(5).start()
        dmod_cols(2, 6)

    def finish_dq(g, dq):
        dq = dq[0:DH, :] * SCALE
        r0 = g * GR if isinstance(g, int) else pl.multiple_of(g * GR, 8)
        dQT[pl.ds(r0, GR), :] = jnp.concatenate([dq[:, 0:TQ], dq[:, TQ:VQ]], axis=0)

    def bwd_body(gg, carry):
        gs = [gg * UB + u for u in range(UB)]
        gp = jnp.maximum(gs[0] - 1, 0)
        qTs = [_ld(QB[i * NG + g]) for g in gs]
        Ws = [_ld(WB[g]) for g in gs]
        nch = S // CKB
        H2 = CKB // 2
        dq = DQ[...]
        prev = (gp, _ld(QB[i * NG + gp]), S - CKB, _ld(DS[...]))
        for u in range(UB):
            for c in range(nch):
                c0 = c * CKB
                pg, pq, pc0, pds = prev
                dpa = _dot(_ld(Vaug[c0 // 2:(c0 + H2) // 2, :]), Ws[u])
                dKT[:, pc0:pc0 + CKB] += _dot_nt(pq, pds)
                dpb = _dot(_ld(Vaug[(c0 + H2) // 2:(c0 + CKB) // 2, :]), Ws[u])
                p = _ld(P[gs[u], c0 // 2:(c0 + CKB) // 2, :])
                dVT[:, c0:c0 + CKB] += _dot_nt(Ws[u], p)
                r = _dot(_ld(KT[:, pc0:pc0 + CKB]), pds)
                dq = r if dq is None else dq + r
                if pc0 + CKB == S:
                    finish_dq(pg, dq)
                    dq = None
                pf = p.astype(F32)
                ds = jnp.concatenate([(pf[:H2] * dpa).astype(BF16), (pf[H2:] * dpb).astype(BF16)], axis=0)
                prev = (gs[u], qTs[u], c0, ds)
        DS[...] = _pk(prev[3])
        DQ[...] = dq
        return carry

    with jax.named_scope('bwdloop'):
        jax.lax.fori_loop(0, NG // UB, bwd_body, 0)

    with jax.named_scope('post'):
        pds = _ld(DS[...])
        dKT[:, S - CKB:S] += _dot_nt(_ld(QB[i * NG + NG - 1]), pds)
        finish_dq(NG - 1, DQ[...] + _dot(_ld(KT[:, S - CKB:S]), pds))
        dQs[...] = _pk(dQT[...].astype(BF16))

    @pl.when(i == NB - 1)
    @jax.named_scope('epilogue')
    def _epilogue():
        dh1T[:, S - TQ:S] = _dot(swq[...], _ld(dQs[...]))
        KT[...] = _pk((dKT[...] * (1.0 / LOG2E)).astype(BF16))
        VT[...] = _pk(dVT[...].astype(BF16))
        ca1 = modc[1]
        eye = _eye(128)

        def ln1b_body(t, carry):
            c0 = pl.multiple_of(t * LW, LW)
            dkvc = jnp.concatenate([_ld(KT[:, pl.ds(c0, LW)]), _ld(VT[:, pl.ds(c0, LW)])], axis=0)
            dh1 = dh1T[:, pl.ds(c0, LW)] + _dot(_ld(wkv[...]), dkvc)
            QR = D // (S // LW)
            q0 = pl.multiple_of(t * QR, 16)
            hq0 = pl.multiple_of(t * (QR // 2), 8)
            swq[pl.ds(q0, QR), :] = (aWq[pl.ds(q0, QR), :] + _dot_nt(
                _ld(h1T[pl.ds(hq0, QR // 2), S - TQ:S]), _ld(dQs[...]))).astype(BF16)
            akv[...] = jnp.where(t > 0, akv[...], 0.0) + _dot_nt(dkvc, _ld(h1T[:, pl.ds(c0, LW)]))
            mu = st1[0:1, pl.ds(c0, LW)]
            rstd = st1[1:2, pl.ds(c0, LW)]
            xh = (_ld(xT[:, pl.ds(c0, LW)]).astype(F32) - mu) * rstd
            macc[1] += _fold(dh1 * xh)
            macc[0] += _fold(dh1)
            dxh1 = dh1 * _wide(ca1, LW)
            n1 = jnp.mean(dxh1, axis=0, keepdims=True)
            n2 = jnp.mean(dxh1 * xh, axis=0, keepdims=True)
            dxt = (dx2T[:, pl.ds(c0, LW)] + rstd * (dxh1 - n1 - xh * n2)).astype(BF16)
            for k in range(LW // 128):
                r0 = pl.multiple_of(t * LW + 128 * k, 128)
                sx[pl.ds(r0, 128), :] = _dot_nt(eye, dxt[:, 128 * k:128 * (k + 1)]).astype(BF16)
            dx_copy(t).start()
            dwq_copy(t).start()
            return carry

        jax.lax.fori_loop(0, S // LW, ln1b_body, 0)
        dwkT_ref[...] = akv[0:DH, :].astype(BF16)
        dwvT_ref[...] = akv[HD:HD + DH, :].astype(BF16)

        dmod_cols(0, 2)
        cf = c_ref[...].astype(F32)
        sgc = _sigmoid(cf)
        dc_ref[...] = (dscs[0:1, :] * (sgc * (1.0 + cf * (1.0 - sgc)))).astype(BF16)
        for k in range(6):
            dwmod_copy(k).wait()
        for t in range(S // LW):
            dx_copy(t).wait()
            dwq_copy(t).wait()
        for k in range(3, 6):
            out_copy(k).wait()


@jax.jit
def pallas_adaLN_cond__grouped_kv_mqa__dense_activation_silu__prompt_kernel(
    A_x: jax.Array,
    A_wq: jax.Array,
    A_wk: jax.Array,
    A_wv: jax.Array,
    A_wo: jax.Array,
    B_x: jax.Array,
    B_w1: jax.Array,
    B_w2: jax.Array,
    c: jax.Array,
    w_mod: jax.Array,
    grad_out: jax.Array,
):
    x = A_x.reshape(S, D)
    g = grad_out.reshape(S, D)

    def full(shape):
        return pl.BlockSpec(shape, lambda i: (0,) * len(shape))

    hbm = pl.BlockSpec(memory_space=pl.ANY)

    in_specs = [
        hbm, hbm, full((DH, D)), full((DH, D)), hbm,
        hbm, hbm, full((1, D)), hbm,
        pl.BlockSpec((TQ, D), lambda i: (i, 0)),
    ]
    out_specs = [
        pl.BlockSpec((TQ, D), lambda i: (i, 0)),
        hbm, hbm, full((DH, D)), full((DH, D)), hbm,
        hbm, hbm, full((1, D)), hbm,
    ]
    out_shape = [
        jax.ShapeDtypeStruct((S, D), BF16), jax.ShapeDtypeStruct((S, D), BF16),
        jax.ShapeDtypeStruct((D, D), BF16), jax.ShapeDtypeStruct((DH, D), BF16),
        jax.ShapeDtypeStruct((DH, D), BF16), jax.ShapeDtypeStruct((D, D), BF16),
        jax.ShapeDtypeStruct((FF, D), BF16), jax.ShapeDtypeStruct((FF, D), BF16),
        jax.ShapeDtypeStruct((1, D), BF16), jax.ShapeDtypeStruct((D, 6 * D), BF16),
    ]
    scratch = [
        pltpu.VMEM((S, D), BF16),
        pltpu.VMEM((D, D), BF16),
        pltpu.VMEM((D, D), BF16),
        pltpu.VMEM((2, FF, D), BF16),
        pltpu.VMEM((D, 6 * D), BF16),
        pltpu.SemaphoreType.DMA((13 + 2 * (S // LW) + 6 + NB,)),
        pltpu.VMEM((D // 2, S), U32),
        pltpu.VMEM((8, S), F32),
        pltpu.VMEM((D // 2, S), U32),
        pltpu.VMEM((6, D, 128), F32),
        pltpu.VMEM((D // 2, D), U32),
        pltpu.VMEM((D // 2, D), U32),
        pltpu.VMEM((2 * NFC, D // 2, FC), U32),
        pltpu.VMEM((D // 2, 2 * HD), U32),
        pltpu.VMEM((S // 2, HD), U32),
        pltpu.VMEM((S // 2, HD), U32),
        pltpu.VMEM((HD // 2, S), U32),
        pltpu.VMEM((HD // 2, S), U32),
        pltpu.VMEM((D + 16, TQ), F32),
        pltpu.VMEM((NB * NG, HD // 2, VQ), U32),
        pltpu.VMEM((D, TQ), F32),
        pltpu.VMEM((D, TQ), F32),
        pltpu.VMEM((D, TQ), F32),
        pltpu.VMEM((S, VQ), F32),
        pltpu.VMEM((S, VQ), F32),
        pltpu.VMEM((8, VQ), F32),
        pltpu.VMEM((8, VQ), F32),
        pltpu.VMEM((NG, S // 2, VQ), U32),
        pltpu.VMEM((NG, 8, VQ), F32),
        pltpu.VMEM((HD, S), F32),
        pltpu.VMEM((HD, S), F32),
        pltpu.VMEM((FF, D), F32),
        pltpu.VMEM((FF, D), F32),
        pltpu.VMEM((D, D), F32),
        pltpu.VMEM((D, D), F32),
        pltpu.VMEM((6, D, 128), F32),
        pltpu.VMEM((D, S), F32),
        pltpu.VMEM((D, S), F32),
        pltpu.VMEM((D // 2, TQ), U32),
        pltpu.VMEM((D // 2, TQ), U32),
        pltpu.VMEM((D, TQ), F32),
        pltpu.VMEM((D, TQ), F32),
        pltpu.SMEM((1,), jnp.int32),
        pltpu.VMEM((NG, HD // 2, VQ), U32),
        pltpu.VMEM((D // 2, TQ), U32),
        pltpu.VMEM((8, D), F32),
        pltpu.VMEM((NG, 24, VQ), F32),
        pltpu.VMEM((CKB // 2, VQ), U32),
        pltpu.VMEM((HD, VQ), F32),
        pltpu.VMEM((2 * HD, D), F32),
    ]
    outs = pl.pallas_call(
        _kernel,
        grid=(NB,),
        in_specs=in_specs,
        out_specs=out_specs,
        out_shape=out_shape,
        scratch_shapes=scratch,
        compiler_params=pltpu.CompilerParams(
            dimension_semantics=("arbitrary",),
            vmem_limit_bytes=126 * 1024 * 1024,
        ),
    )(x, A_wq, A_wk.T, A_wv.T, A_wo, B_w1.T, B_w2, c, w_mod, g)
    out, dx, dwq, dwkT, dwvT, dwo, dw1T, dw2, dc, dwmod = outs
    return (out.reshape(1, S, D), dx.reshape(1, S, D), dwq, dwkT.T, dwvT.T, dwo, dw1T.T, dw2, dc, dwmod)
```

```python
import jax
import jax.numpy as jnp
import jax.experimental.pallas as pl
import jax.experimental.pallas.tpu as pltpu

F32 = jnp.float32
BF16 = jnp.bfloat16
U32 = jnp.uint32

S = 2048
D = 640
H = 32
DH = 20
FF = 1728
FC = 864
NFC = FF // FC
FS = 288
EPS = 1e-5

TQ = 256
NB = S // TQ
HP = 2
NG = H // HP
GR = HP * DH
VQ = HP * TQ
CKF = 128
CKB = 256
HD = 32
UF = 2
UB = 4
SKEW = 1
LW = 512

LOG2E = 1.4426950408889634
SCALE = DH ** (-0.5)

_NT = (((1,), (1,)), ((), ()))


def _dot(a, b):
    return jnp.dot(a, b, preferred_element_type=F32)


def _dot_nt(a, b):
    return jax.lax.dot_general(a, b, _NT, preferred_element_type=F32)


def _ld(v):
    return pltpu.bitcast(v, BF16)


def _pk(v):
    return pltpu.bitcast(v, U32)


def _eye(n, dtype=BF16):
    r = jax.lax.broadcasted_iota(jnp.int32, (n, n), 0)
    c = jax.lax.broadcasted_iota(jnp.int32, (n, n), 1)
    return jnp.where(r == c, 1.0, 0.0).astype(dtype)


def _sigmoid(x):
    return 0.5 * jnp.tanh(0.5 * x) + 0.5


def _wide(col, n):
    reps = n // 128
    if reps == 1:
        return col
    return jnp.concatenate([col] * reps, axis=1)


def _fold(a):
    n = a.shape[1] // 128
    acc = a[:, 0:128]
    for t in range(1, n):
        acc = acc + a[:, t * 128:(t + 1) * 128]
    return acc


def _kernel(x_hbm, wq_hbm, wkT_ref, wvT_ref, wo_hbm, w1T_hbm, w2_hbm, c_ref, wmod_hbm, g_ref,
            out_ref, dx_hbm, dwq_hbm, dwkT_ref, dwvT_ref, dwo_hbm, dw1T_hbm, dw2_hbm, dc_ref, dwmod_hbm,
            sx, swq, swo, sw12, swm, sems,
            xT, st1, h1T, modc, wqT, woT, wT12, wkv,
            Kaug, Vaug, KT, VT, Qs, QB, dOs, OT, dQT, SA, SB, mA, mB, P, linv_s, dKT, dVT,
            aW1, aW2, aWq, aWo, macc, dx2T, dh1T, h2s, dfs, facc, hacc, zs, WB, dQs, dscs, ACC, DS, DQ, akv):
    i = pl.program_id(0)
    sw1 = sw12.at[0]
    sw2 = sw12.at[1]

    in_pairs = [(wmod_hbm, swm), (x_hbm, sx), (wq_hbm, swq), (wo_hbm, swo),
                (w1T_hbm, sw1), (w2_hbm, sw2)]

    def in_copy(k):
        return pltpu.make_async_copy(in_pairs[k][0], in_pairs[k][1], sems.at[k])

    out_pairs = [(swm, dwmod_hbm), (sx, dx_hbm), (swq, dwq_hbm), (swo, dwo_hbm),
                 (sw1, dw1T_hbm), (sw2, dw2_hbm)]

    def out_copy(k):
        return pltpu.make_async_copy(out_pairs[k][0], out_pairs[k][1], sems.at[6 + k])

    def transpose_into(dst, src_ref, ncols):
        nrows = src_ref.shape[0]

        def body(k, carry):
            c0 = pl.multiple_of(k * 128, 128)
            r0 = pl.multiple_of(k * 64, 64)
            dst[pl.ds(r0, 64), 0:nrows] = _pk(_dot_nt(_eye(128), src_ref[:, pl.ds(c0, 128)]).astype(BF16))
            return carry

        jax.lax.fori_loop(0, ncols // 128, body, 0)

    def cast_rows(dst, src, nrows, blk):
        def body(k, carry):
            r0 = pl.multiple_of(k * blk, blk)
            dst[pl.ds(r0, blk), :] = src[pl.ds(r0, blk), :].astype(BF16)
            return carry

        jax.lax.fori_loop(0, nrows // blk, body, 0)

    def wmod_copy(part):
        lo, hi = (0, 2 * D) if part == 0 else (2 * D, 6 * D)
        return pltpu.make_async_copy(wmod_hbm.at[:, lo:hi], swm.at[:, lo:hi], sems.at[0 if part == 0 else 12])

    def dwmod_copy(k):
        c0 = k * D if isinstance(k, int) else pl.multiple_of(k * D, 128)
        return pltpu.make_async_copy(swm.at[:, pl.ds(c0, D)], dwmod_hbm.at[:, pl.ds(c0, D)],
                                     sems.at[13 + S // LW + k])

    def x_copy(b):
        r0 = b * TQ if isinstance(b, int) else pl.multiple_of(b * TQ, TQ)
        return pltpu.make_async_copy(x_hbm.at[pl.ds(r0, TQ), :], sx.at[pl.ds(r0, TQ), :],
                                     sems.at[13 + S // LW + 6 + b])

    def dwq_copy(t):
        QR = D // (S // LW)
        r0 = t * QR if isinstance(t, int) else pl.multiple_of(t * QR, 16)
        return pltpu.make_async_copy(swq.at[pl.ds(r0, QR), :], dwq_hbm.at[pl.ds(r0, QR), :],
                                     sems.at[13 + S // LW + 6 + NB + t])

    def dx_copy(t):
        r0 = t * LW if isinstance(t, int) else pl.multiple_of(t * LW, LW)
        return pltpu.make_async_copy(sx.at[pl.ds(r0, LW), :], dx_hbm.at[pl.ds(r0, LW), :], sems.at[13 + t])

    def dmod_cols(k_lo, k_hi):
        cf = c_ref[...].astype(F32)
        sc = cf * _sigmoid(cf)
        scc = jnp.transpose(jnp.broadcast_to(sc, (128, D)))
        rid = jax.lax.broadcasted_iota(jnp.int32, (16, D), 0)

        def body(k, carry):
            c0 = pl.multiple_of(k * D, 128)
            row = jnp.sum(jnp.transpose(macc[k]), axis=0, keepdims=True)
            hi = row.astype(BF16).astype(F32)
            lo = row - hi
            lhs = jnp.where(rid == 0, hi, jnp.where(rid == 1, lo, 0.0)).astype(BF16)
            d2 = _dot_nt(lhs, swm[:, pl.ds(c0, D)])
            swm[:, pl.ds(c0, D)] = (_wide(scc, D) * row).astype(BF16)
            dscs[0:1, :] += d2[0:1] + d2[1:2]
            dwmod_copy(k).start()
            return carry

        jax.lax.fori_loop(k_lo, k_hi, body, 0)

    def mod_col(k):
        cf = c_ref[...].astype(F32)
        sc = cf * _sigmoid(cf)
        scb = jnp.broadcast_to(sc, (16, D)).astype(BF16)
        c0 = k * D if isinstance(k, int) else pl.multiple_of(k * D, 128)
        row = _dot(scb, swm[:, pl.ds(c0, D)])[0:1]
        row = row + jnp.where(jnp.logical_or(k == 1, k == 4), 1.0, 0.0)
        modc[k] = jnp.transpose(jnp.broadcast_to(row, (128, D)))

    def mod_cols(k_lo, k_hi):
        def body(k, carry):
            mod_col(k)
            return carry

        jax.lax.fori_loop(k_lo, k_hi, body, 0)

    def score_pass(n, Snext, mnext, c, m8):
        c0 = c * CKF
        z = pl.multiple_of(zs[0], 8)
        qT = _ld(QB[n])
        s = _dot(_ld(Kaug[c0 // 2:(c0 + CKF) // 2, :]), qT)
        Snext[pl.ds(z + c0, CKF), :] = s
        mc = jnp.max(s.reshape(CKF // 8, 8, VQ), axis=0)
        return mc if m8 is None else jnp.maximum(m8, mc)

    @pl.when(i == 0)
    @jax.named_scope('prologue')
    def _prologue():
        wmod_copy(0).start()
        x_copy(0).start()
        in_copy(2).start()
        for b in range(1, NB):
            x_copy(b).start()
        zs[0] = 0

        macc[...] = jnp.zeros_like(macc)
        dKT[...] = jnp.zeros_like(dKT)
        dVT[...] = jnp.zeros_like(dVT)
        dQT[...] = jnp.zeros_like(dQT)
        DS[...] = jnp.zeros_like(DS)
        DQ[...] = jnp.zeros_like(DQ)
        dscs[...] = jnp.zeros_like(dscs)
        Qs[D:D + 16, :] = jnp.zeros((16, TQ), F32)

        z12 = jnp.zeros((HD - DH, D), F32)
        wkvT = jnp.concatenate([wkT_ref[...].astype(F32), z12, wvT_ref[...].astype(F32), z12],
                               axis=0).astype(BF16)
        eye128 = _eye(128)
        for c0 in range(0, D, 128):
            wkv[c0 // 2:(c0 + 128) // 2, :] = _pk(_dot_nt(eye128, wkvT[:, c0:c0 + 128]).astype(BF16))

        wmod_copy(0).wait()
        mod_cols(0, 2)

        rowid = jax.lax.broadcasted_iota(jnp.int32, (HD, TQ), 0)
        ones_rows = jnp.logical_and(rowid >= DH, rowid < DH + 2)

        def ln1_block(t):
            t0 = pl.multiple_of(t * TQ, TQ)
            xt = jnp.transpose(sx[pl.ds(t0, TQ), :].astype(F32))
            xT[:, pl.ds(t0, TQ)] = _pk(xt.astype(BF16))
            mu = jnp.mean(xt, axis=0, keepdims=True)
            xc = xt - mu
            var = jnp.mean(xc * xc, axis=0, keepdims=True)
            rstd = jax.lax.rsqrt(var + EPS)
            st1[0:1, pl.ds(t0, TQ)] = mu
            st1[1:2, pl.ds(t0, TQ)] = rstd
            h1 = (xc * rstd * _wide(modc[1], TQ) + _wide(modc[0], TQ)).astype(BF16)
            h1T[:, pl.ds(t0, TQ)] = _pk(h1)
            kv = _dot(wkvT, h1)
            kt = kv[0:HD].astype(BF16)
            vt = jnp.where(ones_rows, 1.0, kv[HD:2 * HD]).astype(BF16)
            KT[:, pl.ds(t0, TQ)] = _pk(kt)
            VT[:, pl.ds(t0, TQ)] = _pk(vt)
            for k in range(TQ // 128):
                r0 = pl.multiple_of(t * (TQ // 2) + 64 * k, 64)
                Kaug[pl.ds(r0, 64), :] = _pk(_dot_nt(eye128, kt[:, 128 * k:128 * (k + 1)]).astype(BF16))
                Vaug[pl.ds(r0, 64), :] = _pk(_dot_nt(eye128, vt[:, 128 * k:128 * (k + 1)]).astype(BF16))

        def q_block(b):
            t0 = pl.multiple_of(b * TQ, TQ)
            Qs[0:D, :] = _dot(_ld(wqT[...]), _ld(h1T[:, pl.ds(t0, TQ)])) * (SCALE * LOG2E)
            for g in range(NG):
                qblk = Qs[g * GR:g * GR + GR + 16, :]
                qT = jnp.concatenate([qblk[0:HD], qblk[DH:DH + HD]], axis=1).astype(BF16)
                QB[b * NG + g] = _pk(qT)

        x_copy(0).wait()
        ln1_block(zs[0])
        in_copy(2).wait()
        in_copy(4).start()
        in_copy(5).start()
        in_copy(3).start()
        wmod_copy(1).start()
        transpose_into(wqT, swq, D)

        def pq_body(b, carry):
            x_copy(b + 1).wait()
            q_block(b)
            ln1_block(jnp.minimum(b + 1, NB - 1))
            return carry

        NW = 2 * NFC
        jax.lax.fori_loop(0, NB - NW, pq_body, 0)

        in_copy(4).wait()

        def pq2_body(b, carry):
            k = b - (NB - NW)

            @pl.when(k == NFC)
            def _():
                in_copy(5).wait()

            @pl.when(b + 1 < NB)
            def _():
                x_copy(b + 1).wait()

            q_block(b)
            ln1_block(jnp.minimum(b + 1, NB - 1))
            r0 = pl.multiple_of((k % NFC) * FC, 32)
            for c0 in range(0, D, 128):
                wT12[k, c0 // 2:(c0 + 128) // 2, :] = _pk(
                    jnp.transpose(sw12[k // NFC, pl.ds(r0, FC), c0:c0 + 128]))
            return carry

        jax.lax.fori_loop(NB - NW, NB, pq2_body, 0)

        in_copy(3).wait()
        wmod_copy(1).wait()
        for c0 in range(0, D, 128):
            woT[c0 // 2:(c0 + 128) // 2, :] = _pk(jnp.transpose(swo[:, c0:c0 + 128]))
        for k in range(2, 6):
            mod_col(k)
        m8 = None
        for c in range(S // CKF):
            m8 = score_pass(0, SA, mA, c, m8)
        mA[...] = m8


    t0 = pl.multiple_of(i * TQ, TQ)

    def fwd_step(g, n, Scur, mcur, Snext, mnext):
        m = jnp.max(mcur[...], axis=0, keepdims=True)
        z = pl.multiple_of(zs[0], 8)
        m8 = None
        acc = None
        nch = S // CKF
        for cc in range(nch + SKEW):
            if cc < nch:
                m8 = score_pass(n, Snext, mnext, cc, m8)
            if cc >= SKEW:
                c0 = (cc - SKEW) * CKF
                p = jnp.exp2(Scur[pl.ds(z + c0, CKF), :] - m).astype(BF16)
                P[g, c0 // 2:(c0 + CKF) // 2, :] = _pk(p)
                r = _dot(_ld(VT[:, c0:c0 + CKF]), p)
                acc = r if acc is None else acc + r
        mnext[...] = m8
        ACC[g] = acc[0:24, :]

    def fwd_body(gg, carry):
        g = UF * gg
        n = i * NG + g
        for u in range(0, UF, 2):
            fwd_step(g + u, n + u + 1, SA, mA, SB, mB)
            fwd_step(g + u + 1, jnp.minimum(n + u + 2, NB * NG - 1), SB, mB, SA, mA)
        return carry

    with jax.named_scope('fwdloop'):
        jax.lax.fori_loop(0, NG // UF, fwd_body, 0)

    def finish_dq(g, dq):
        dq = dq[0:DH, :] * SCALE
        r0 = g * GR if isinstance(g, int) else pl.multiple_of(g * GR, 8)
        dQT[pl.ds(r0, GR), :] = jnp.concatenate([dq[:, 0:TQ], dq[:, TQ:VQ]], axis=0)

    def bwd_tail(blk):
        pds = _ld(DS[...])
        dKT[:, S - CKB:S] += _dot_nt(_ld(QB[blk * NG + NG - 1]), pds)
        finish_dq(NG - 1, DQ[...] + _dot(_ld(KT[:, S - CKB:S]), pds))
        dQs[...] = _pk(dQT[...].astype(BF16))

    with jax.named_scope('mid1'):
        ga = _wide(modc[2], TQ)
        sb = _wide(modc[3], TQ)
        cb1 = _wide(modc[4], TQ)
        gb = _wide(modc[5], TQ)

        gT = jnp.transpose(g_ref[...].astype(F32))
        dfs[...] = _pk((gT * gb).astype(BF16))

        for g in range(NG):
            acc = ACC[g]
            linv = 1.0 / acc[DH:DH + 1, :]
            linv_s[g] = jnp.broadcast_to(linv, (8, VQ))
            o = acc[0:DH, :] * linv
            OT[g * GR:(g + 1) * GR, :] = jnp.concatenate([o[:, 0:TQ], o[:, TQ:VQ]], axis=0)
        ip = jnp.maximum(i - 1, 0)
        tp = pl.multiple_of(ip * TQ, TQ)
        bwd_tail(ip)
        OTb = OT[...].astype(BF16)
        attn = _dot(_ld(woT[...]), OTb)
        h1p = _ld(h1T[:, pl.ds(tp, TQ)])
        dQp = _ld(dQs[...])
        aWq[...] = jnp.where(i > 0, aWq[...], 0.0) + _dot_nt(h1p, dQp)
        x2 = _ld(xT[:, pl.ds(t0, TQ)]).astype(F32) + ga * attn
        mu2 = jnp.mean(x2, axis=0, keepdims=True)
        xc2 = x2 - mu2
        var2 = jnp.mean(xc2 * xc2, axis=0, keepdims=True)
        rstd2 = jax.lax.rsqrt(var2 + EPS)
        xh2 = xc2 * rstd2
        h2s[...] = _pk((xh2 * cb1 + sb).astype(BF16))

    def ffn_body(j, carry):
        h2 = _ld(h2s[...])
        df = _ld(dfs[...])
        a_parts = []
        du_parts = []
        for sb_ in range(FC // FS):
            f0 = pl.multiple_of(j * FC + sb_ * FS, 32)
            u = _dot(sw1[pl.ds(f0, FS), :], h2)
            da = _dot(sw2[pl.ds(f0, FS), :], df)
            sg = _sigmoid(u)
            a = (u * sg).astype(BF16)
            du = (da * (sg * (1.0 + u * (1.0 - sg)))).astype(BF16)
            aW2[pl.ds(f0, FS), :] = jnp.where(i > 0, aW2[pl.ds(f0, FS), :], 0.0) + _dot_nt(a, df)
            aW1[pl.ds(f0, FS), :] = jnp.where(i > 0, aW1[pl.ds(f0, FS), :], 0.0) + _dot_nt(du, h2)
            a_parts.append(a)
            du_parts.append(du)
        a = jnp.concatenate(a_parts, axis=0)
        du = jnp.concatenate(du_parts, axis=0)
        facc[...] = jnp.where(j > 0, facc[...], 0.0) + _dot(_ld(wT12[NFC + j]), a)
        hacc[...] = jnp.where(j > 0, hacc[...], 0.0) + _dot(_ld(wT12[j]), du)
        return carry

    with jax.named_scope('ffnloop'):
        jax.lax.fori_loop(0, NFC, ffn_body, 0)

    with jax.named_scope('mid2'):
        dh1T[:, pl.ds(tp, TQ)] = _dot(swq[...], _ld(dQs[...]))
        f = facc[...]
        outT = (x2 + gb * f).astype(BF16)
        out_ref[...] = jnp.transpose(outT)
        macc[5] += _fold(gT * f)
        dh2 = hacc[...]
        macc[4] += _fold(dh2 * xh2)
        macc[3] += _fold(dh2)
        dxh = dh2 * cb1
        m1 = jnp.mean(dxh, axis=0, keepdims=True)
        m2 = jnp.mean(dxh * xh2, axis=0, keepdims=True)
        dx2 = gT + rstd2 * (dxh - m1 - xh2 * m2)
        dx2T[:, pl.ds(t0, TQ)] = dx2
        macc[2] += _fold(dx2 * attn)
        dattn = (dx2 * ga).astype(BF16)
        dOs[...] = _dot(swo[...], dattn)
        aWo[...] = jnp.where(i > 0, aWo[...], 0.0) + _dot_nt(OTb, dattn)
        for g in range(NG):
            dob = dOs[g * GR:(g + 1) * GR, :]
            ob = OT[g * GR:(g + 1) * GR, :]
            do = jnp.concatenate([dob[0:DH], dob[DH:GR]], axis=1)
            o = jnp.concatenate([ob[0:DH], ob[DH:GR]], axis=1)
            linv = linv_s[g][0:1, :]
            nd = -jnp.sum(do * o, axis=0, keepdims=True) * linv
            nd_hi = nd.astype(BF16).astype(F32)
            nd_lo = nd - nd_hi
            W = jnp.concatenate([do * linv, nd_hi, nd_lo, jnp.zeros((HD - DH - 2, VQ), F32)],
                                axis=0).astype(BF16)
            WB[g] = _pk(W)
        DS[...] = jnp.zeros_like(DS)
        DQ[...] = jnp.zeros_like(DQ)

    @pl.when(i == NB - 1)
    @jax.named_scope('earlyout')
    def _early_out():
        cast_rows(swo, aWo, D, 64)
        cast_rows(sw1, aW1, FF, 64)
        cast_rows(sw2, aW2, FF, 64)
        out_copy(3).start()
        out_copy(4).start()
        out_copy(5).start()
        dmod_cols(2, 6)

    def bwd_body(gg, carry):
        gs = [gg * UB + u for u in range(UB)]
        gp = jnp.maximum(gs[0] - 1, 0)
        qTs = [_ld(QB[i * NG + g]) for g in gs]
        Ws = [_ld(WB[g]) for g in gs]
        nch = S // CKB
        H2 = CKB // 2
        dq = DQ[...]
        prev = (gp, _ld(QB[i * NG + gp]), S - CKB, _ld(DS[...]))
        for u in range(UB):
            for c in range(nch):
                c0 = c * CKB
                pg, pq, pc0, pds = prev
                dpa = _dot(_ld(Vaug[c0 // 2:(c0 + H2) // 2, :]), Ws[u])
                dKT[:, pc0:pc0 + CKB] += _dot_nt(pq, pds)
                dpb = _dot(_ld(Vaug[(c0 + H2) // 2:(c0 + CKB) // 2, :]), Ws[u])
                p = _ld(P[gs[u], c0 // 2:(c0 + CKB) // 2, :])
                dVT[:, c0:c0 + CKB] += _dot_nt(Ws[u], p)
                r = _dot(_ld(KT[:, pc0:pc0 + CKB]), pds)
                dq = r if dq is None else dq + r
                if pc0 + CKB == S:
                    finish_dq(pg, dq)
                    dq = None
                pf = p.astype(F32)
                ds = jnp.concatenate([(pf[:H2] * dpa).astype(BF16), (pf[H2:] * dpb).astype(BF16)], axis=0)
                prev = (gs[u], qTs[u], c0, ds)
        DS[...] = _pk(prev[3])
        DQ[...] = dq
        return carry

    with jax.named_scope('bwdloop'):
        jax.lax.fori_loop(0, NG // UB, bwd_body, 0)

    @pl.when(i == NB - 1)
    @jax.named_scope('epilogue')
    def _epilogue():
        bwd_tail(NB - 1)
        dh1T[:, S - TQ:S] = _dot(swq[...], _ld(dQs[...]))
        KT[...] = _pk((dKT[...] * (1.0 / LOG2E)).astype(BF16))
        VT[...] = _pk(dVT[...].astype(BF16))
        ca1 = modc[1]
        eye = _eye(128)

        def ln1b_body(t, carry):
            c0 = pl.multiple_of(t * LW, LW)
            dkvc = jnp.concatenate([_ld(KT[:, pl.ds(c0, LW)]), _ld(VT[:, pl.ds(c0, LW)])], axis=0)
            dh1 = dh1T[:, pl.ds(c0, LW)] + _dot(_ld(wkv[...]), dkvc)
            QR = D // (S // LW)
            q0 = pl.multiple_of(t * QR, 16)
            hq0 = pl.multiple_of(t * (QR // 2), 8)
            swq[pl.ds(q0, QR), :] = (aWq[pl.ds(q0, QR), :] + _dot_nt(
                _ld(h1T[pl.ds(hq0, QR // 2), S - TQ:S]), _ld(dQs[...]))).astype(BF16)
            akv[...] = jnp.where(t > 0, akv[...], 0.0) + _dot_nt(dkvc, _ld(h1T[:, pl.ds(c0, LW)]))
            mu = st1[0:1, pl.ds(c0, LW)]
            rstd = st1[1:2, pl.ds(c0, LW)]
            xh = (_ld(xT[:, pl.ds(c0, LW)]).astype(F32) - mu) * rstd
            macc[1] += _fold(dh1 * xh)
            macc[0] += _fold(dh1)
            dxh1 = dh1 * _wide(ca1, LW)
            n1 = jnp.mean(dxh1, axis=0, keepdims=True)
            n2 = jnp.mean(dxh1 * xh, axis=0, keepdims=True)
            dxt = (dx2T[:, pl.ds(c0, LW)] + rstd * (dxh1 - n1 - xh * n2)).astype(BF16)
            for k in range(LW // 128):
                r0 = pl.multiple_of(t * LW + 128 * k, 128)
                sx[pl.ds(r0, 128), :] = _dot_nt(eye, dxt[:, 128 * k:128 * (k + 1)]).astype(BF16)
            dx_copy(t).start()
            dwq_copy(t).start()
            return carry

        jax.lax.fori_loop(0, S // LW, ln1b_body, 0)
        dwkT_ref[...] = akv[0:DH, :].astype(BF16)
        dwvT_ref[...] = akv[HD:HD + DH, :].astype(BF16)

        dmod_cols(0, 2)
        cf = c_ref[...].astype(F32)
        sgc = _sigmoid(cf)
        dc_ref[...] = (dscs[0:1, :] * (sgc * (1.0 + cf * (1.0 - sgc)))).astype(BF16)
        for k in range(6):
            dwmod_copy(k).wait()
        for t in range(S // LW):
            dx_copy(t).wait()
            dwq_copy(t).wait()
        for k in range(3, 6):
            out_copy(k).wait()


@jax.jit
def pallas_adaLN_cond__grouped_kv_mqa__dense_activation_silu__prompt_kernel(
    A_x: jax.Array,
    A_wq: jax.Array,
    A_wk: jax.Array,
    A_wv: jax.Array,
    A_wo: jax.Array,
    B_x: jax.Array,
    B_w1: jax.Array,
    B_w2: jax.Array,
    c: jax.Array,
    w_mod: jax.Array,
    grad_out: jax.Array,
):
    x = A_x.reshape(S, D)
    g = grad_out.reshape(S, D)

    def full(shape):
        return pl.BlockSpec(shape, lambda i: (0,) * len(shape))

    hbm = pl.BlockSpec(memory_space=pl.ANY)

    in_specs = [
        hbm, hbm, full((DH, D)), full((DH, D)), hbm,
        hbm, hbm, full((1, D)), hbm,
        pl.BlockSpec((TQ, D), lambda i: (i, 0)),
    ]
    out_specs = [
        pl.BlockSpec((TQ, D), lambda i: (i, 0)),
        hbm, hbm, full((DH, D)), full((DH, D)), hbm,
        hbm, hbm, full((1, D)), hbm,
    ]
    out_shape = [
        jax.ShapeDtypeStruct((S, D), BF16), jax.ShapeDtypeStruct((S, D), BF16),
        jax.ShapeDtypeStruct((D, D), BF16), jax.ShapeDtypeStruct((DH, D), BF16),
        jax.ShapeDtypeStruct((DH, D), BF16), jax.ShapeDtypeStruct((D, D), BF16),
        jax.ShapeDtypeStruct((FF, D), BF16), jax.ShapeDtypeStruct((FF, D), BF16),
        jax.ShapeDtypeStruct((1, D), BF16), jax.ShapeDtypeStruct((D, 6 * D), BF16),
    ]
    scratch = [
        pltpu.VMEM((S, D), BF16),
        pltpu.VMEM((D, D), BF16),
        pltpu.VMEM((D, D), BF16),
        pltpu.VMEM((2, FF, D), BF16),
        pltpu.VMEM((D, 6 * D), BF16),
        pltpu.SemaphoreType.DMA((13 + 2 * (S // LW) + 6 + NB,)),
        pltpu.VMEM((D // 2, S), U32),
        pltpu.VMEM((8, S), F32),
        pltpu.VMEM((D // 2, S), U32),
        pltpu.VMEM((6, D, 128), F32),
        pltpu.VMEM((D // 2, D), U32),
        pltpu.VMEM((D // 2, D), U32),
        pltpu.VMEM((2 * NFC, D // 2, FC), U32),
        pltpu.VMEM((D // 2, 2 * HD), U32),
        pltpu.VMEM((S // 2, HD), U32),
        pltpu.VMEM((S // 2, HD), U32),
        pltpu.VMEM((HD // 2, S), U32),
        pltpu.VMEM((HD // 2, S), U32),
        pltpu.VMEM((D + 16, TQ), F32),
        pltpu.VMEM((NB * NG, HD // 2, VQ), U32),
        pltpu.VMEM((D, TQ), F32),
        pltpu.VMEM((D, TQ), F32),
        pltpu.VMEM((D, TQ), F32),
        pltpu.VMEM((S, VQ), F32),
        pltpu.VMEM((S, VQ), F32),
        pltpu.VMEM((8, VQ), F32),
        pltpu.VMEM((8, VQ), F32),
        pltpu.VMEM((NG, S // 2, VQ), U32),
        pltpu.VMEM((NG, 8, VQ), F32),
        pltpu.VMEM((HD, S), F32),
        pltpu.VMEM((HD, S), F32),
        pltpu.VMEM((FF, D), F32),
        pltpu.VMEM((FF, D), F32),
        pltpu.VMEM((D, D), F32),
        pltpu.VMEM((D, D), F32),
        pltpu.VMEM((6, D, 128), F32),
        pltpu.VMEM((D, S), F32),
        pltpu.VMEM((D, S), F32),
        pltpu.VMEM((D // 2, TQ), U32),
        pltpu.VMEM((D // 2, TQ), U32),
        pltpu.VMEM((D, TQ), F32),
        pltpu.VMEM((D, TQ), F32),
        pltpu.SMEM((1,), jnp.int32),
        pltpu.VMEM((NG, HD // 2, VQ), U32),
        pltpu.VMEM((D // 2, TQ), U32),
        pltpu.VMEM((8, D), F32),
        pltpu.VMEM((NG, 24, VQ), F32),
        pltpu.VMEM((CKB // 2, VQ), U32),
        pltpu.VMEM((HD, VQ), F32),
        pltpu.VMEM((2 * HD, D), F32),
    ]
    outs = pl.pallas_call(
        _kernel,
        grid=(NB,),
        in_specs=in_specs,
        out_specs=out_specs,
        out_shape=out_shape,
        scratch_shapes=scratch,
        compiler_params=pltpu.CompilerParams(
            dimension_semantics=("arbitrary",),
            vmem_limit_bytes=126 * 1024 * 1024,
        ),
    )(x, A_wq, A_wk.T, A_wv.T, A_wo, B_w1.T, B_w2, c, w_mod, g)
    out, dx, dwq, dwkT, dwvT, dwo, dw1T, dw2, dc, dwmod = outs
    return (out.reshape(1, S, D), dx.reshape(1, S, D), dwq, dwkT.T, dwvT.T, dwo, dw1T.T, dw2, dc, dwmod)
```
